```python
import os as _os
_os.environ.setdefault('JAX_PLATFORMS', 'cpu')
import jax
import jax.numpy as jnp

def _softmax(x, axis=-1):
    return jax.nn.softmax(x, axis=axis)

def _gelu(x):
    return jax.nn.gelu(x, approximate=True)

def _silu(x):
    return jax.nn.silu(x)

def _sigmoid(x):
    return jax.nn.sigmoid(x)

def _layernorm(x, axis=-1, eps=1e-05):
    m = jnp.mean(x, axis=axis, keepdims=True)
    v = jnp.var(x, axis=axis, keepdims=True)
    return (x - m) / jnp.sqrt(v + eps)

def _scatter_add(tgt, idx, src, axis=0):
    return tgt.at[idx].add(src)

def _segment_sum(src, seg, n):
    return jax.ops.segment_sum(src, seg, n)

class _Rng:

    def __init__(self, key):
        self._k = key

    def _next(self):
        self._k, sub = jax.random.split(self._k)
        return sub

    def normal(self, shape):
        return jax.random.normal(self._next(), shape, dtype=jnp.bfloat16)

    def randint(self, lo, hi, shape):
        return jax.random.randint(self._next(), shape, lo, hi, dtype=jnp.int32)

    def uniform(self, shape, lo=0.0, hi=1.0):
        return jax.random.uniform(self._next(), shape, jnp.bfloat16, lo, hi)

    def permutation(self, n):
        return jax.random.permutation(self._next(), n)
kernel_name = 'adaLN_cond__sliding_local_dilated__dense_activation_relu__prompt'

def setup_inputs():
    _rng = _Rng(jax.random.key(int.from_bytes(__import__("os").urandom(4), "little")))
    _w = lambda a: (lambda t: t.astype(jnp.bfloat16) if jnp.issubdtype(t.dtype, jnp.floating) else t)(jnp.asarray(a))

    def _A_setup():
        B, S, D = (1, 2048, 576)
        return {'x': _w((lambda *s: _rng.normal(s) * 0.05)(B, S, D)), 'wqkv': _w((lambda *s: _rng.normal(s) * 0.05)(D, 3 * D)), 'wo': _w((lambda *s: _rng.normal(s) * 0.05)(D, D))}
    _A_in = _A_setup()

    def _B_setup():
        B, S, D, Dff = (1, 2048, 576, 4608)
        return {'x': _w((lambda *s: _rng.normal(s) * 0.05)(B, S, D)), 'w1': _w((lambda *s: _rng.normal(s) * 0.05)(D, Dff)), 'w2': _w((lambda *s: _rng.normal(s) * 0.05)(Dff, D))}
    _B_in = _B_setup()
    return {'A_x': _A_in['x'], 'A_wqkv': _A_in['wqkv'], 'A_wo': _A_in['wo'], 'B_x': _B_in['x'], 'B_w1': _B_in['w1'], 'B_w2': _B_in['w2'], 'c': _w((lambda *s: _rng.normal(s) * 0.05)(1, 576) * 8.0), 'w_mod': _w((lambda *s: _rng.normal(s) * 0.05)(576, 6 * 576) * 576 ** (-0.5) * 8.0)}

def reference(A_x, A_wqkv, A_wo, B_x, B_w1, B_w2, c, w_mod):

    def _A_ref(x, wqkv, wo):
        B, S, D = x.shape
        H = 32
        Dh = D // H
        W, dil = (8, 2)
        qkv = (lambda x, *d: x.transpose(*d))((x @ wqkv).reshape(B, S, 3, H, Dh), 2, 0, 3, 1, 4)
        q, k, v = (qkv[0], qkv[1], qkv[2])
        scale = Dh ** (-0.5)
        pos = jnp.arange(S)
        off = jnp.arange(W) * dil
        idx = pos[:, None] - off[None, :]
        mask = idx >= 0
        idx_c = jnp.where(mask, idx, 0).reshape(-1)
        kg = k[:, :, idx_c, :].reshape(B, H, S, W, Dh)
        vg = v[:, :, idx_c, :].reshape(B, H, S, W, Dh)
        logits = jnp.einsum('bhsd,bhswd->bhsw', q, kg) * scale
        logits = jnp.where(mask[None, None, :, :], logits, -1000000000.0)
        attn = _softmax(logits, axis=-1)
        o = jnp.einsum('bhsw,bhswd->bhsd', attn, vg)
        return (lambda x, *d: x.transpose(*d))(o, 0, 2, 1, 3).reshape(B, S, D) @ wo

    def _B_ref(x, w1, w2):
        h = jnp.einsum('bsd,df->bsf', x, w1)
        zero = jnp.zeros_like(h)
        h = jnp.maximum(h, zero)
        return jnp.einsum('bsf,fd->bsd', h, w2)
    x = A_x
    mod = (_silu(c) @ w_mod).reshape(c.shape[0], 6, 1, -1)
    sa, ca, ga, sb, cb, gb = (mod[:, 0].copy(), mod[:, 1].copy(), mod[:, 2].copy(), mod[:, 3].copy(), mod[:, 4].copy(), mod[:, 5].copy())
    h = _layernorm(x, axis=-1) * (1 + ca) + sa
    x = x + ga * _A_ref(h, A_wqkv, A_wo)
    h = _layernorm(x, axis=-1) * (1 + cb) + sb
    x = x + gb * _B_ref(h, B_w1, B_w2)
    return x
```

```python
import math
import jax, jax.numpy as jnp, numpy as np
from jax import lax
from jax.experimental import pallas as pl
from jax.experimental.pallas import tpu as pltpu

S, D, DFF = 2048, 576, 4608
H, DH, W, DIL = 32, 18, 8, 2
DP = 640
NQ = 14
HALO = 16
EPS = 1e-5
NT = (((1,), (1,)), ((), ()))
F32, BF16 = jnp.float32, jnp.bfloat16

def nt_dot(a, b):
    return lax.dot_general(a, b, NT, preferred_element_type=F32)

def qkv_row(part, d):
    if d < 16:
        return 128 * (4 * part + d // 4) + 32 * (d % 4)
    t = d - 16
    if part == 0:
        return 128 * 12 + 32 * t
    if part == 1:
        return 128 * 13 + 32 * t
    return 128 * 13 + 64 + 32 * t

Q_SLABS = (0, 1, 2, 3, 12)
K_SLABS = (4, 5, 6, 7, 13)
V_SLABS = (8, 9, 10, 11, 13)
QT = (0, 1, 2, 3, 12)
KVT = (4, 5, 6, 7, 8, 9, 10, 11, 13)
FLAGS = {None: None,
         'lp': {'XLA_TPU_FORCE_LP_LLO_SCHEDULER': True},
         'even': {'XLA_TPU_EVENLY_DISTRIBUTE_CRITICAL_NODES': True},
         'res': {'XLA_TPU_RESCHEDULE_DMA_DONES': True},
         'evenres': {'XLA_TPU_EVENLY_DISTRIBUTE_CRITICAL_NODES': True, 'XLA_TPU_RESCHEDULE_DMA_DONES': True},
         'evenlp': {'XLA_TPU_EVENLY_DISTRIBUTE_CRITICAL_NODES': True, 'XLA_TPU_FORCE_LP_LLO_SCHEDULER': True}}

def make(TM=256, FC=512, NA=16, jc=6, flags=None, skew=True, opq=3, modi=2, b1=True, scopes=False, TA=256, pc=4, lnr=1, ln1r=0, qs=True, w5=7, nsplit=3, outmode=1, slab=False, swp=True, serwo=False):
    nblk = S // TM
    na = S // TA

    def lanes(v, n):
        return jnp.concatenate([v] * (n // 128), axis=1) if n > 128 else v

    def ln_mod_T(xT, scale1p, shift, reload=None, fence=None):
        n = xT.shape[1]
        m = jnp.mean(xT, axis=0, keepdims=True)
        if reload is None:
            xc = xT - m
            v = jnp.mean(xc * xc, axis=0, keepdims=True)
        else:
            xc = reload() - m
            v = jnp.mean(xc * xc, axis=0, keepdims=True)
            fence(v)
            xc = reload() - m
        hT = (xc * lax.rsqrt(v + EPS)) * lanes(scale1p, n) + lanes(shift, n)
        hT = jnp.concatenate([hT.astype(BF16), jnp.zeros((DP - D, n), BF16)], axis=0)
        return hT.T

    import contextlib
    def scope(name):
        return jax.named_scope(name) if scopes else contextlib.nullcontext()

    def kernel(c_hbm, xT_hbm, wqkv_hbm, wo_hbm, w1_hbm, w2T_hbm, wmod_hbm, outT_hbm,
               c_v, xT_v, wqkv_v, wo_v, w1p, w2T_v, wmod_v, wT_f, wp, woT, modT, qkv, qkv0, hb1, hb2, x1T, ost,
               a0, zero_s, zsem, sems):
        cp = lambda src, dst, k: pltpu.make_async_copy(src, dst, sems.at[k])
        xs = lambda lo, hi, k: cp(xT_hbm.at[:, lo:hi], xT_v.at[:, lo:hi], k)
        grp1 = [cp(c_hbm, c_v, 0), cp(wmod_hbm.at[:, 0:1152], wmod_v.at[:, 0:1152], 1)]
        grp2 = [cp(wqkv_hbm.at[:, 0:640], wqkv_v.at[:, 0:640], 2)]
        grp2b = [xs(0, TA, 3)]
        grp2c = [xs(TA, 3 * TA, 13)]
        grp3 = [cp(wqkv_hbm.at[:, 640:1728], wqkv_v.at[:, 640:1728], 4), xs(3 * TA, 4 * TA, 5)]
        grp4 = [xs(4 * TA, S, 6), cp(wo_hbm, wo_v, 7), cp(wmod_hbm.at[:, 1152:3456], wmod_v.at[:, 1152:3456], 8)]
        if slab:
            grp5 = ([cp(w1_hbm.at[:, 128 * t:128 * t + 128], w1p.at[t, 0:D, :], 9) for t in range(36)] +
                    [cp(w2T_hbm.at[:, 128 * t:128 * t + 128], w2T_v.at[t], 10) for t in range(36)])
        else:
            grp5 = [cp(w1_hbm, w1p.at[0:D, :], 9), cp(w2T_hbm, w2T_v, 10)]
        for g in (grp1, grp2, grp2b, grp2c, grp3, grp4, grp5):
            for d in g:
                d.start()
        def wait(g, name):
            with scope(name):
                for d in g:
                    d.wait()

        zero_s[0] = 0
        if slab:
            w1p[:, D:DP, :] = jnp.zeros((36, DP - D, 128), BF16)
        else:
            w1p[D:DP, :] = jnp.zeros((DP - D, DFF), BF16)
        for j in KVT:
            qkv0[j, 0:HALO, :] = jnp.zeros((HALO, 128), F32)
        if swp:
            wp[:, 128 * 12 + 64:128 * 13, :] = jnp.zeros((5, 64, 128), BF16)
        else:
            wp[128 * 12 + 64:128 * 13, :] = jnp.zeros((64, DP), BF16)

        wait(grp1, "wait1")
        cc = c_v[...].astype(F32)
        s16 = jnp.broadcast_to(cc * jax.nn.sigmoid(cc), (16, D)).astype(BF16)
        def mod_tiles(t0, t1):
            m = jnp.dot(s16, wmod_v[:, 128 * t0:128 * t1], preferred_element_type=F32)
            for t in range(t1 - t0):
                row = jnp.broadcast_to(m[0:1, 128 * t:128 * t + 128], (128, 128))
                modT[128 * (t0 + t):128 * (t0 + t + 1), :] = row.T
        mod_tiles(0, 9)

        def w_transpose(c0, c1):
            for j in range(5):
                lo = 128 * j
                n = min(128, D - lo)
                blk = wqkv_v[lo:lo + n, c0:c1]
                if n < 128:
                    blk = jnp.concatenate([blk, jnp.zeros((128 - n, c1 - c0), BF16)], axis=0)
                wT_f[j, c0:c1, :] = blk.T.astype(F32)
        def w_regroup(part):
            for d in range(DH):
                r = qkv_row(part, d)
                for j in range(5):
                    v = wT_f.at[j][pl.ds(D * part + d, 32, stride=DH), :].astype(BF16)
                    if swp:
                        wp[j, r:r + 32, :] = v
                    else:
                        wp[r:r + 32, 128 * j:128 * j + 128] = v

        def ln_a(i):
            ld = lambda: xT_v[:, i * TA:(i + 1) * TA].astype(F32)
            if ln1r:
                def fence(v):
                    x1T[0, D:D + 8, 0:TA] = jnp.broadcast_to(v, (8, TA))
                hb1[i] = ln_mod_T(ld(), 1.0 + modT[D:2 * D, :], modT[0:D, :], ld, fence)
            else:
                hb1[i] = ln_mod_T(ld(), 1.0 + modT[D:2 * D, :], modT[0:D, :])
        def mm_a(i, tiles, between=None):
            h = hb1[i]
            for j in tiles:
                if swp:
                    wt = jnp.concatenate([wp[k, 128 * j:128 * j + 128, :] for k in range(5)], axis=1)
                else:
                    wt = wp[128 * j:128 * j + 128, :]
                r = nt_dot(h, wt)
                if qs and j in QT:
                    r = r * ((DH ** -0.5) * math.log2(math.e))
                if (i + 1) * TA <= TM:
                    qkv0[j, HALO + i * TA:HALO + (i + 1) * TA, :] = r
                    if j in KVT and (i + 1) * TA == TM:
                        qkv[j, TM:HALO + TM, :] = r[TA - HALO:TA, :]
                else:
                    qkv[j, HALO + i * TA:HALO + (i + 1) * TA, :] = r
                if between is not None:
                    between()

        def prep_wo():
            for t in range(5):
                lo = 128 * t
                n = min(128, D - lo)
                u = 0 if serwo else t
                wT_f[u, 0:D, 0:n] = wo_v[:, lo:lo + n].astype(F32)
                parts = [wT_f.at[u][pl.ds(d, 32, stride=DH), 0:n] for d in range(16)]
                parts.append(jnp.zeros((64, n), F32))
                parts += [wT_f.at[u][pl.ds(d, 32, stride=DH), 0:n] for d in (16, 17)]
                blk = jnp.concatenate(parts, axis=0).astype(BF16)
                woT[lo:lo + n, :] = blk.T

        c2 = (DH ** -0.5) * math.log2(math.e)

        def stage_b(i, qkv_, obase):
            static = isinstance(i, int)
            base = i * TM
            for ch in range(TM // NA):
                t0 = base + ch * NA
                r0 = HALO + t0
                if not static:
                    r0 = pl.multiple_of(r0, 8)
                qs = [qkv_[j, pl.ds(r0, NA), :] for j in Q_SLABS]
                logits = []
                for w in range(W):
                    rw = r0 - DIL * w
                    acc = None
                    for qi, j in enumerate(K_SLABS):
                        p = qs[qi] * qkv_[j, pl.ds(rw, NA), :]
                        acc = p if acc is None else acc + p
                    acc = acc + pltpu.roll(acc, 64, 1)
                    acc = acc + pltpu.roll(acc, 32, 1)
                    if ch * NA < DIL * w:
                        tok = t0 + lax.broadcasted_iota(jnp.int32, (NA, 128), 0)
                        acc = jnp.where(tok >= DIL * w, acc, -1e9)
                    logits.append(acc)
                m = logits[0]
                for w in range(1, W):
                    m = jnp.maximum(m, logits[w])
                ps = [jnp.exp2((l - m) if qs else (l - m) * c2) for l in logits]
                den = ps[0]
                for w in range(1, W):
                    den = den + ps[w]
                r = pltpu.reciprocal(den, approx=True)
                inv = r * (2.0 - den * r)
                for vi, j in enumerate(V_SLABS):
                    acc = None
                    for w in range(W):
                        p = ps[w] * qkv_[j, pl.ds(r0 - DIL * w, NA), :]
                        acc = p if acc is None else acc + p
                    qkv_[NQ + vi, pl.ds(obase + ch * NA, NA), :] = acc * inv

        def stage_c(i, slot, qkv_, obase):
            o = jnp.concatenate([qkv_[NQ + vi, pl.ds(obase, TM), :] for vi in range(5)], axis=1).astype(BF16)
            attnT = nt_dot(woT[...], o)
            if isinstance(i, int):
                xT = xT_v[:, i * TM:(i + 1) * TM]
            else:
                xT = xT_v[:, pl.ds(pl.multiple_of(i * TM, 128), TM)]
            x1 = xT.astype(F32) + lanes(modT[2 * D:3 * D, :], TM) * attnT
            x1T[slot, 0:D, :] = x1
            if lnr:
                def fence(v):
                    x1T[slot, D:D + 8, :] = jnp.broadcast_to(v, (8, TM))
                hb2[slot] = ln_mod_T(x1, 1.0 + modT[4 * D:5 * D, :], modT[3 * D:4 * D, :], lambda: x1T[slot, 0:D, :], fence)
            else:
                hb2[slot] = ln_mod_T(x1, 1.0 + modT[4 * D:5 * D, :], modT[3 * D:4 * D, :])

        def cp_out(i, slot):
            if isinstance(i, int):
                dst = outT_hbm.at[:, i * TM:(i + 1) * TM]
            else:
                dst = outT_hbm.at[:, pl.ds(pl.multiple_of(i * TM, 128), TM)]
            if outmode >= 1:
                return pltpu.make_async_copy(ost.at[i], dst, sems.at[11])
            return pltpu.make_async_copy(ost.at[slot], dst, sems.at[11 + slot])

        def mm1(h, j):
            if slab:
                wt = jnp.concatenate([w1p[j * (FC // 128) + t] for t in range(FC // 128)], axis=1)
            else:
                wt = w1p[:, j * FC:(j + 1) * FC]
            h1 = jnp.dot(h, wt, preferred_element_type=F32)
            return jnp.maximum(h1, 0.0).astype(BF16)

        def first_chunk(slot):
            a0[...] = mm1(hb2[slot], 0)

        def stage_d(i, slot, hooks={}):
            h = hb2[slot]
            nj = DFF // FC
            acc = None
            a_next = a0[...]
            for j in range(nj):
                a = a_next
                if j + 1 < nj:
                    a_next = mm1(h, j + 1)
                if j in hooks:
                    hooks[j]()
                if slab:
                    wt = jnp.concatenate([w2T_v[j * (FC // 128) + t] for t in range(FC // 128)], axis=1)
                else:
                    wt = w2T_v[:, j * FC:(j + 1) * FC]
                p = nt_dot(wt, a)
                acc = p if acc is None else acc + p
            ost[i if outmode >= 1 else slot] = (x1T[slot, 0:D, :] + lanes(modT[5 * D:6 * D, :], TM) * acc).astype(BF16)

        wait(grp2, "wait2")
        w_transpose(0, 640)
        w_regroup(0)
        wait(grp2b, "wait2b")
        ln_a(0)
        mm_a(0, QT[:nsplit])
        wait(grp2c, "wait2c")
        ln_a(1)
        ln_a(2)
        mm_a(0, QT[nsplit:])
        mm_a(1, QT)
        wait(grp3, "wait3")
        w_transpose(640, 1728)
        w_regroup(1)
        w_regroup(2)
        ln_a(3)
        mm_a(2, QT)
        mm_a(3, QT)
        mm_a(0, KVT)
        mm_a(1, KVT)
        wait(grp4, "wait4")
        if opq == 1:
            ob0 = pl.multiple_of(zero_s[0], 8)
        elif opq == 3:
            ob0 = pl.multiple_of(pl.semaphore_read(zsem) * 8, 8)
        else:
            ob0 = 0
        stage_b(0, qkv0, ob0)
        prep_wo()
        todo = [t for t in range(9, 27)]
        def mod_next():
            if todo:
                ts = todo[:modi]
                del todo[:modi]
                mod_tiles(ts[0], ts[-1] + 1)
        if modi == 0:
            mod_tiles(9, 27)
            todo.clear()
        mm_a(2, KVT, mod_next)
        mm_a(3, KVT, mod_next)
        for i in range(4, na):
            ln_a(i)
            if i == w5:
                wait(grp5, "wait5")
            mm_a(i, tuple(range(NQ)), mod_next)
            if i == pc:
                assert not todo
                stage_c(0, 0, qkv0, ob0)
        if w5 >= na:
            wait(grp5, "wait5")
        first_chunk(0)

        def body(i, _):
            slot = i % 2
            if outmode == 0:
                @pl.when(i >= 2)
                def _():
                    cp_out(i - 2, slot).wait()
            ob = pl.multiple_of((1 - slot) * TM, 8)
            stage_b(i + 1, qkv, ob)
            stage_d(i, slot, {jc: lambda: stage_c(i + 1, 1 - slot, qkv, ob)})
            first_chunk(1 - slot)
            if outmode <= 1:
                cp_out(i, slot).start()
            return 0
        lax.fori_loop(0, nblk - 1, body, 0)
        last = nblk - 1
        if outmode == 0:
            with scope("waitM"):
                cp_out(last - 2, last % 2).wait()
        stage_d(last, last % 2)
        cp_out(last, last % 2).start()
        if outmode == 2:
            for i in range(last):
                cp_out(i, 0).start()
        with scope("wait6"):
            if outmode == 0:
                cp_out(last - 1, (last - 1) % 2).wait()
                cp_out(last, last % 2).wait()
            else:
                for i in range(nblk):
                    cp_out(i, 0).wait()

    def f(A_x, A_wqkv, A_wo, B_x, B_w1, B_w2, c, w_mod):
        xT = A_x.reshape(S, D).T
        any_spec = pl.BlockSpec(memory_space=pl.ANY)
        outT = pl.pallas_call(
            kernel,
            grid=(1,) if opq == 2 else (),
            in_specs=[any_spec] * 7,
            out_specs=any_spec,
            out_shape=jax.ShapeDtypeStruct((D, S), BF16),
            scratch_shapes=[
                pltpu.VMEM((1, D), BF16),
                pltpu.VMEM((D, S), BF16),
                pltpu.VMEM((D, 3 * D), BF16),
                pltpu.VMEM((D, D), BF16),
                pltpu.VMEM((36, DP, 128) if slab else (DP, DFF), BF16),
                pltpu.VMEM((36, D, 128) if slab else (D, DFF), BF16),
                pltpu.VMEM((D, 6 * D), BF16),
                pltpu.VMEM((5, 3 * D, 128), F32),
                pltpu.VMEM((5, 128 * NQ, 128) if swp else (128 * NQ, DP), BF16),
                pltpu.VMEM((D, DP), BF16),
                pltpu.VMEM((6 * D, 128), F32),
                pltpu.VMEM((NQ + 5, HALO + S, 128), F32),
                pltpu.VMEM((NQ + 5, HALO + TM, 128), F32),
                pltpu.VMEM((na, TA, DP), BF16),
                pltpu.VMEM((2, TM, DP), BF16),
                pltpu.VMEM((2, D + 8, TM), F32),
                pltpu.VMEM((nblk if outmode else 2, D, TM), BF16),
                pltpu.VMEM((TM, FC), BF16),
                pltpu.SMEM((1,), jnp.int32),
                pltpu.SemaphoreType.REGULAR,
                pltpu.SemaphoreType.DMA((14,)),
            ],
            compiler_params=pltpu.CompilerParams(vmem_limit_bytes=100 * 1024 * 1024, flags=FLAGS[flags]),
        )(c, xT, A_wqkv, A_wo, B_w1, B_w2.T, w_mod)
        return outT.T.reshape(1, S, D)
    return f


_kernel_fn = make(TM=256, flags='even', pc=5)

@jax.jit
def pallas_adaLN_cond__sliding_local_dilated__dense_activation_relu__prompt_kernel(A_x, A_wqkv, A_wo, B_x, B_w1, B_w2, c, w_mod):
    return _kernel_fn(A_x, A_wqkv, A_wo, B_x, B_w1, B_w2, c, w_mod)
```

```python
import math
import jax, jax.numpy as jnp, numpy as np
from jax import lax
from jax.experimental import pallas as pl
from jax.experimental.pallas import tpu as pltpu

S, D, DFF = 2048, 576, 4608
H, DH, W, DIL = 32, 18, 8, 2
DP = 640
NQ = 14
HALO = 16
EPS = 1e-5
NT = (((1,), (1,)), ((), ()))
F32, BF16 = jnp.float32, jnp.bfloat16

def nt_dot(a, b):
    return lax.dot_general(a, b, NT, preferred_element_type=F32)

def qkv_row(part, d):
    if d < 16:
        return 128 * (4 * part + d // 4) + 32 * (d % 4)
    t = d - 16
    if part == 0:
        return 128 * 12 + 32 * t
    if part == 1:
        return 128 * 13 + 32 * t
    return 128 * 13 + 64 + 32 * t

Q_SLABS = (0, 1, 2, 3, 12)
K_SLABS = (4, 5, 6, 7, 13)
V_SLABS = (8, 9, 10, 11, 13)
QT = (0, 1, 2, 3, 12)
KVT = (4, 5, 6, 7, 8, 9, 10, 11, 13)
FLAGS = {None: None,
         'lp': {'XLA_TPU_FORCE_LP_LLO_SCHEDULER': True},
         'even': {'XLA_TPU_EVENLY_DISTRIBUTE_CRITICAL_NODES': True},
         'res': {'XLA_TPU_RESCHEDULE_DMA_DONES': True},
         'evenres': {'XLA_TPU_EVENLY_DISTRIBUTE_CRITICAL_NODES': True, 'XLA_TPU_RESCHEDULE_DMA_DONES': True},
         'evenlp': {'XLA_TPU_EVENLY_DISTRIBUTE_CRITICAL_NODES': True, 'XLA_TPU_FORCE_LP_LLO_SCHEDULER': True}}

def make(TM=256, FC=512, NA=16, jc=6, flags=None, skew=True, opq=3, modi=2, b1=True, scopes=False, TA=256, pc=4, lnr=1, ln1r=0, qs=True, w5=7, nsplit=3, outmode=1, slab=False, swp=True, serwo=False, cps=True, order=1, n3=0, x3e=True, n4=0, b4=2, x4e=True, nochk=True, rot=True, pre1=True, lsplit=False):
    nblk = S // TM
    na = S // TA

    def lanes(v, n):
        return jnp.concatenate([v] * (n // 128), axis=1) if n > 128 else v

    def ln_mod_T(xT, scale1p, shift, reload=None, fence=None):
        n = xT.shape[1]
        m = jnp.mean(xT, axis=0, keepdims=True)
        if reload is None:
            xc = xT - m
            v = jnp.mean(xc * xc, axis=0, keepdims=True)
        else:
            xc = reload() - m
            v = jnp.mean(xc * xc, axis=0, keepdims=True)
            fence(v)
            xc = reload() - m
        hT = (xc * lax.rsqrt(v + EPS)) * lanes(scale1p, n) + lanes(shift, n)
        hT = jnp.concatenate([hT.astype(BF16), jnp.zeros((DP - D, n), BF16)], axis=0)
        return hT.T

    def kvs(j, p):
        if not cps or p == 0:
            return j
        return NQ + 5 + 3 * KVT.index(j) + (p - 1)
    NSL = NQ + 5 + (27 if cps else 0)
    PADR = 8 if cps else 0
    import contextlib
    def scope(name):
        return jax.named_scope(name) if scopes else contextlib.nullcontext()

    def kernel(c_hbm, xT_hbm, wqkv_hbm, wo_hbm, w1_hbm, w2T_hbm, wmod_hbm, outT_hbm,
               c_v, xT_v, wqkv_v, wo_v, w1p, w2T_v, wmod_v, wT_f, wp, woT, modT, qkv, qkv0, hb1, hb2, x1T, ost,
               a0, zero_s, zsem, sems):
        cp = lambda src, dst, k: pltpu.make_async_copy(src, dst, sems.at[k])
        xs = lambda lo, hi, k: cp(xT_hbm.at[:, lo:hi], xT_v.at[:, lo:hi], k)
        grp1 = [cp(c_hbm, c_v, 0), cp(wmod_hbm.at[:, 0:1152], wmod_v.at[:, 0:1152], 1)]
        grp2 = [cp(wqkv_hbm.at[:, 0:640], wqkv_v.at[:, 0:640], 2)]
        grp2b = [xs(0, TA, 3)]
        if x3e:
            grp2c = [xs(TA, 4 * TA, 13)]
            grp3 = [cp(wqkv_hbm.at[:, 640:1728], wqkv_v.at[:, 640:1728], 4)]
            if x4e:
                grp3.append(xs(4 * TA, 5 * TA, 5))
        else:
            grp2c = [xs(TA, 3 * TA, 13)]
            grp3 = [cp(wqkv_hbm.at[:, 640:1728], wqkv_v.at[:, 640:1728], 4), xs(3 * TA, 4 * TA, 5)]
        grp4 = [xs((5 if x4e else 4) * TA, S, 6), cp(wo_hbm, wo_v, 7), cp(wmod_hbm.at[:, 1152:3456], wmod_v.at[:, 1152:3456], 8)]
        if slab:
            grp5 = ([cp(w1_hbm.at[:, 128 * t:128 * t + 128], w1p.at[t, 0:D, :], 9) for t in range(36)] +
                    [cp(w2T_hbm.at[:, 128 * t:128 * t + 128], w2T_v.at[t], 10) for t in range(36)])
        else:
            grp5 = [cp(w1_hbm, w1p.at[0:D, :], 9), cp(w2T_hbm, w2T_v, 10)]
        for g in ((grp1, grp2) if order == 0 else (grp2, grp1)) + (grp2b, grp2c, grp3, grp4, grp5):
            for d in g:
                d.start()
        def wait(g, name):
            with scope(name):
                for d in g:
                    d.wait()

        zero_s[0] = 0
        if slab:
            w1p[:, D:DP, :] = jnp.zeros((36, DP - D, 128), BF16)
        else:
            w1p[D:DP, :] = jnp.zeros((DP - D, DFF), BF16)
        for j in KVT:
            for p in range(4 if cps else 1):
                qkv0[kvs(j, p), 0:HALO + (8 if p else 0), :] = jnp.zeros((HALO + (8 if p else 0), 128), F32)
        if swp:
            wp[:, 128 * 12 + 64:128 * 13, :] = jnp.zeros((5, 64, 128), BF16)
        else:
            wp[128 * 12 + 64:128 * 13, :] = jnp.zeros((64, DP), BF16)

        s16 = None
        def mod_tiles(t0, t1):
            m = jnp.dot(s16, wmod_v[:, 128 * t0:128 * t1], preferred_element_type=F32)
            for t in range(t1 - t0):
                row = jnp.broadcast_to(m[0:1, 128 * t:128 * t + 128], (128, 128))
                col = row.T
                if pre1:
                    n0 = 128 * (t0 + t)
                    if (n0 < 2 * D and n0 + 128 > D) or (n0 < 5 * D and n0 + 128 > 4 * D):
                        rid = n0 + lax.broadcasted_iota(jnp.int32, (128, 128), 0)
                        isc = ((rid >= D) & (rid < 2 * D)) | ((rid >= 4 * D) & (rid < 5 * D))
                        col = jnp.where(isc, col + 1.0, col)
                modT[128 * (t0 + t):128 * (t0 + t + 1), :] = col

        def w_transpose(c0, c1):
            for j in range(5):
                lo = 128 * j
                n = min(128, D - lo)
                blk = wqkv_v[lo:lo + n, c0:c1]
                if n < 128:
                    blk = jnp.concatenate([blk, jnp.zeros((128 - n, c1 - c0), BF16)], axis=0)
                wT_f[j, c0:c1, :] = blk.T.astype(F32)
        def w_regroup(part):
            for d in range(DH):
                r = qkv_row(part, d)
                for j in range(5):
                    v = wT_f.at[j][pl.ds(D * part + d, 32, stride=DH), :].astype(BF16)
                    if swp:
                        wp[j, r:r + 32, :] = v
                    else:
                        wp[r:r + 32, 128 * j:128 * j + 128] = v

        def ln_a(i):
            ld = lambda: xT_v[:, i * TA:(i + 1) * TA].astype(F32)
            if ln1r:
                def fence(v):
                    x1T[0, D:D + 8, 0:TA] = jnp.broadcast_to(v, (8, TA))
                hb1[i] = ln_mod_T(ld(), (modT[D:2 * D, :] if pre1 else 1.0 + modT[D:2 * D, :]), modT[0:D, :], ld, fence)
            else:
                hb1[i] = ln_mod_T(ld(), (modT[D:2 * D, :] if pre1 else 1.0 + modT[D:2 * D, :]), modT[0:D, :])
        def mm_a(i, tiles, between=None):
            h = hb1[i]
            for j in tiles:
                if swp:
                    wt = jnp.concatenate([wp[k, 128 * j:128 * j + 128, :] for k in range(5)], axis=1)
                else:
                    wt = wp[128 * j:128 * j + 128, :]
                r = nt_dot(h, wt)
                if qs and j in QT:
                    r = r * ((DH ** -0.5) * math.log2(math.e))
                if (i + 1) * TA <= TM:
                    for p in range(4 if (cps and j in KVT) else 1):
                        qkv0[kvs(j, p), HALO + i * TA + 2 * p:HALO + (i + 1) * TA + 2 * p, :] = r
                        if j in KVT and (i + 1) * TA == TM:
                            qkv[kvs(j, p), TM + 2 * p:HALO + TM + 2 * p, :] = r[TA - HALO:TA, :]
                else:
                    for p in range(4 if (cps and j in KVT) else 1):
                        qkv[kvs(j, p), HALO + i * TA + 2 * p:HALO + (i + 1) * TA + 2 * p, :] = r
                if between is not None:
                    between()

        def prep_wo():
            for t in range(5):
                lo = 128 * t
                n = min(128, D - lo)
                u = 0 if serwo else t
                wT_f[u, 0:D, 0:n] = wo_v[:, lo:lo + n].astype(F32)
                parts = [wT_f.at[u][pl.ds(d, 32, stride=DH), 0:n] for d in range(16)]
                parts.append(jnp.zeros((64, n), F32))
                parts += [wT_f.at[u][pl.ds(d, 32, stride=DH), 0:n] for d in (16, 17)]
                blk = jnp.concatenate(parts, axis=0).astype(BF16)
                woT[lo:lo + n, :] = blk.T

        c2 = (DH ** -0.5) * math.log2(math.e)

        def stage_b(i, qkv_, obase):
            static = isinstance(i, int)
            base = i * TM
            for ch in range(TM // NA):
                t0 = base + ch * NA
                r0 = HALO + t0
                if not static:
                    r0 = pl.multiple_of(r0, 8)
                qs = [qkv_[j, pl.ds(r0, NA), :] for j in Q_SLABS]
                def win(j, w):
                    if cps:
                        return qkv_[kvs(j, w % 4), pl.ds(r0 - 8 * (w // 4), NA), :]
                    return qkv_[j, pl.ds(r0 - DIL * w, NA), :]
                logits = []
                for w in range(W):
                    acc = None
                    for qi, j in enumerate(K_SLABS):
                        p = qs[qi] * win(j, w)
                        acc = p if acc is None else acc + p
                    acc = acc + pltpu.roll(acc, 64, 1)
                    acc = acc + pltpu.roll(acc, 32, 1)
                    if ch * NA < DIL * w:
                        tok = t0 + lax.broadcasted_iota(jnp.int32, (NA, 128), 0)
                        acc = jnp.where(tok >= DIL * w, acc, -1e9)
                    logits.append(acc)
                m = logits[0]
                for w in range(1, W):
                    m = jnp.maximum(m, logits[w])
                ps = [jnp.exp2((l - m) if qs else (l - m) * c2) for l in logits]
                den = ps[0]
                for w in range(1, W):
                    den = den + ps[w]
                r = pltpu.reciprocal(den, approx=True)
                inv = r * (2.0 - den * r)
                for vi, j in enumerate(V_SLABS):
                    acc = None
                    for w in range(W):
                        p = ps[w] * win(j, w)
                        acc = p if acc is None else acc + p
                    qkv_[NQ + vi, pl.ds(obase + ch * NA, NA), :] = acc * inv

        def stage_c(i, slot, qkv_, obase):
            o = jnp.concatenate([qkv_[NQ + vi, pl.ds(obase, TM), :] for vi in range(5)], axis=1).astype(BF16)
            attnT = nt_dot(woT[...], o)
            if isinstance(i, int):
                xT = xT_v[:, i * TM:(i + 1) * TM]
            else:
                xT = xT_v[:, pl.ds(pl.multiple_of(i * TM, 128), TM)]
            x1 = xT.astype(F32) + lanes(modT[2 * D:3 * D, :], TM) * attnT
            x1T[slot, 0:D, :] = x1
            if lnr:
                def fence(v):
                    x1T[slot, D:D + 8, :] = jnp.broadcast_to(v, (8, TM))
                hb2[slot] = ln_mod_T(x1, (modT[4 * D:5 * D, :] if pre1 else 1.0 + modT[4 * D:5 * D, :]), modT[3 * D:4 * D, :], lambda: x1T[slot, 0:D, :], fence)
            else:
                hb2[slot] = ln_mod_T(x1, (modT[4 * D:5 * D, :] if pre1 else 1.0 + modT[4 * D:5 * D, :]), modT[3 * D:4 * D, :])

        def cp_out(i, slot):
            if isinstance(i, int):
                dst = outT_hbm.at[:, i * TM:(i + 1) * TM]
            else:
                dst = outT_hbm.at[:, pl.ds(pl.multiple_of(i * TM, 128), TM)]
            if outmode >= 1:
                return pltpu.make_async_copy(ost.at[i], dst, sems.at[11])
            return pltpu.make_async_copy(ost.at[slot], dst, sems.at[11 + slot])

        def mm1(h, j):
            if slab:
                wt = jnp.concatenate([w1p[j * (FC // 128) + t] for t in range(FC // 128)], axis=1)
            else:
                wt = w1p[:, j * FC:(j + 1) * FC]
            h1 = jnp.dot(h, wt, preferred_element_type=F32)
            return jnp.maximum(h1, 0.0).astype(BF16)

        def first_chunk(slot):
            a0[...] = mm1(hb2[slot], 0)

        def stage_d(i, slot, hooks={}):
            h = hb2[slot]
            nj = DFF // FC
            acc = None
            a_next = a0[...] if rot else mm1(h, 0)
            for j in range(nj):
                a = a_next
                if j + 1 < nj:
                    a_next = mm1(h, j + 1)
                if j in hooks:
                    hooks[j]()
                if slab:
                    wt = jnp.concatenate([w2T_v[j * (FC // 128) + t] for t in range(FC // 128)], axis=1)
                else:
                    wt = w2T_v[:, j * FC:(j + 1) * FC]
                p = nt_dot(wt, a)
                acc = p if acc is None else acc + p
            ost[i if outmode >= 1 else slot] = (x1T[slot, 0:D, :] + lanes(modT[5 * D:6 * D, :], TM) * acc).astype(BF16)

        def do_mod0():
            nonlocal s16
            wait(grp1, "wait1")
            cc = c_v[...].astype(F32)
            s16 = jnp.broadcast_to(cc * jax.nn.sigmoid(cc), (16, D)).astype(BF16)
            mod_tiles(0, 9)
        def do_prepq():
            wait(grp2, "wait2")
            w_transpose(0, 640)
            w_regroup(0)
        if order == 0:
            do_mod0(); do_prepq()
        else:
            do_prepq(); do_mod0()
        wait(grp2b, "wait2b")
        ln_a(0)
        mm_a(0, QT[:nsplit])
        wait(grp2c, "wait2c")
        ln_a(1)
        ln_a(2)
        mm_a(0, QT[nsplit:])
        mm_a(1, QT)
        if x3e:
            ln_a(3)
        mm_a(2, QT[:n3])
        if x3e:
            mm_a(3, QT[:n4])
        wait(grp3, "wait3")
        w_transpose(640, 1728)
        w_regroup(1)
        w_regroup(2)
        if not x3e:
            ln_a(3)
        mm_a(2, QT[n3:])
        mm_a(3, QT[n4:] if x3e else QT)
        if x4e:
            ln_a(4)
        for i in range(b4):
            mm_a(i, KVT)
        wait(grp4, "wait4")
        if opq == 1:
            ob0 = pl.multiple_of(zero_s[0], 8)
        elif opq == 3:
            ob0 = pl.multiple_of(pl.semaphore_read(zsem) * 8, 8)
        else:
            ob0 = 0
        stage_b(0, qkv0, ob0)
        prep_wo()
        todo = [t for t in range(9, 27)]
        def mod_next():
            if todo:
                ts = todo[:modi]
                del todo[:modi]
                mod_tiles(ts[0], ts[-1] + 1)
        if modi == 0:
            mod_tiles(9, 27)
            todo.clear()
        for i in range(b4, 4):
            mm_a(i, KVT, mod_next)
        for i in range(4, na):
            if not (x4e and i == 4):
                ln_a(i)
            if i == w5:
                wait(grp5, "wait5")
            mm_a(i, tuple(range(NQ)), mod_next)
            if i == pc:
                assert not todo
                stage_c(0, 0, qkv0, ob0)
        if w5 >= na:
            wait(grp5, "wait5")
        if rot:
            first_chunk(0)

        def mark(name):
            if scopes:
                with scope(name):
                    pl.semaphore_signal(zsem, 1)
                    pl.semaphore_wait(zsem, 1)
        def body(i, _):
            mark("waitL")
            slot = i % 2
            if outmode == 0:
                @pl.when(i >= 2)
                def _():
                    cp_out(i - 2, slot).wait()
            ob = pl.multiple_of((1 - slot) * TM, 8)
            stage_b(i + 1, qkv, ob)
            stage_d(i, slot, {jc: lambda: stage_c(i + 1, 1 - slot, qkv, ob)})
            if rot:
                first_chunk(1 - slot)
            if outmode <= 1:
                cp_out(i, slot).start()
            return 0
        lax.fori_loop(0, nblk - 1, body, 0)
        last = nblk - 1
        mark("waitM")
        if outmode == 0:
            with scope("waitM"):
                cp_out(last - 2, last % 2).wait()
        if lsplit:
            h = hb2[last % 2]
            nj = DFF // FC
            accs = [None, None]
            a_next = mm1(h, 0)
            half = lambda v, u: v[:, 128 * u:128 * u + 128]
            def fin(u):
                res = x1T[last % 2, 0:D, 128 * u:128 * u + 128] + modT[5 * D:6 * D, :] * accs[u]
                ost[last, :, 128 * u:128 * u + 128] = res.astype(BF16)
                pltpu.make_async_copy(ost.at[last, :, 128 * u:128 * u + 128],
                                      outT_hbm.at[:, last * TM + 128 * u:last * TM + 128 * u + 128], sems.at[12]).start()
            for j in range(nj):
                a = a_next
                if j + 1 < nj:
                    a_next = mm1(h, j + 1)
                w2 = w2T_v[:, j * FC:(j + 1) * FC]
                if j + 1 < nj:
                    p = nt_dot(w2, a)
                    for u in range(2):
                        accs[u] = half(p, u) if accs[u] is None else accs[u] + half(p, u)
                else:
                    for u in range(2):
                        accs[u] = accs[u] + nt_dot(w2, a[128 * u:128 * u + 128, :])
                        fin(u)
        else:
            stage_d(last, last % 2)
            cp_out(last, last % 2).start()
        if outmode == 2:
            for i in range(last):
                cp_out(i, 0).start()
        with scope("wait6"):
            if outmode == 0:
                cp_out(last - 1, (last - 1) % 2).wait()
                cp_out(last, last % 2).wait()
            else:
                for i in range(nblk - 1 if lsplit else nblk):
                    cp_out(i, 0).wait()
                if lsplit:
                    for u in range(2):
                        pltpu.make_async_copy(ost.at[last, :, 128 * u:128 * u + 128],
                                              outT_hbm.at[:, last * TM + 128 * u:last * TM + 128 * u + 128], sems.at[12]).wait()

    def f(A_x, A_wqkv, A_wo, B_x, B_w1, B_w2, c, w_mod):
        xT = A_x.reshape(S, D).T
        any_spec = pl.BlockSpec(memory_space=pl.ANY)
        outT = pl.pallas_call(
            kernel,
            grid=(1,) if opq == 2 else (),
            in_specs=[any_spec] * 7,
            out_specs=any_spec,
            out_shape=jax.ShapeDtypeStruct((D, S), BF16),
            scratch_shapes=[
                pltpu.VMEM((1, D), BF16),
                pltpu.VMEM((D, S), BF16),
                pltpu.VMEM((D, 3 * D), BF16),
                pltpu.VMEM((D, D), BF16),
                pltpu.VMEM((36, DP, 128) if slab else (DP, DFF), BF16),
                pltpu.VMEM((36, D, 128) if slab else (D, DFF), BF16),
                pltpu.VMEM((D, 6 * D), BF16),
                pltpu.VMEM((5, 3 * D, 128), F32),
                pltpu.VMEM((5, 128 * NQ, 128) if swp else (128 * NQ, DP), BF16),
                pltpu.VMEM((D, DP), BF16),
                pltpu.VMEM((6 * D, 128), F32),
                pltpu.VMEM((NSL, HALO + S + PADR, 128), F32),
                pltpu.VMEM((NSL, HALO + TM + PADR, 128), F32),
                pltpu.VMEM((na, TA, DP), BF16),
                pltpu.VMEM((2, TM, DP), BF16),
                pltpu.VMEM((2, D + 8, TM), F32),
                pltpu.VMEM((nblk if outmode else 2, D, TM), BF16),
                pltpu.VMEM((TM, FC), BF16),
                pltpu.SMEM((1,), jnp.int32),
                pltpu.SemaphoreType.REGULAR,
                pltpu.SemaphoreType.DMA((14,)),
            ],
            compiler_params=pltpu.CompilerParams(vmem_limit_bytes=100 * 1024 * 1024, flags=FLAGS[flags], disable_semaphore_checks=nochk, disable_bounds_checks=nochk),
        )(c, xT, A_wqkv, A_wo, B_w1, B_w2.T, w_mod)
        return outT.T.reshape(1, S, D)
    return f


_kernel_fn = make(flags='even', n3=5, pc=5, w5=8, rot=False, jc=6, lsplit=True)

@jax.jit
def pallas_adaLN_cond__sliding_local_dilated__dense_activation_relu__prompt_kernel(A_x, A_wqkv, A_wo, B_x, B_w1, B_w2, c, w_mod):
    return _kernel_fn(A_x, A_wqkv, A_wo, B_x, B_w1, B_w2, c, w_mod)
```

```python
import math

import jax
import jax.numpy as jnp
from jax import lax
from jax.experimental import pallas as pl
from jax.experimental.pallas import tpu as pltpu

S, D, DFF = 2048, 576, 4608
H, DH, W, DIL = 32, 18, 8, 2
EPS = 1e-5
DP = 640
TM = 256
NB = S // TM
FC = 512
NA = 16
HALO = 16
LOG2E = math.log2(math.e)
F32, BF16 = jnp.float32, jnp.bfloat16

NQ = 14
QT = (0, 1, 2, 3, 12)
KT = (4, 5, 6, 7, 13)
VT = (8, 9, 10, 11, 13)
KVT = (4, 5, 6, 7, 8, 9, 10, 11, 13)
NSL = NQ + 5 + 3 * len(KVT)


def _nt_dot(a, b):
    return lax.dot_general(a, b, (((1,), (1,)), ((), ())), preferred_element_type=F32)


def _qkv_row(part, d):
    if d < 16:
        return 128 * (4 * part + d // 4) + 32 * (d % 4)
    return (128 * 12, 128 * 13, 128 * 13 + 64)[part] + 32 * (d - 16)


def _kv_slab(j, p):
    return j if p == 0 else NQ + 5 + 3 * KVT.index(j) + (p - 1)


def _lanes(v, n):
    return jnp.concatenate([v] * (n // 128), axis=1)


def _ln_mod(xT, scale1p, shift, reload=None, fence=None):
    m = jnp.mean(xT, axis=0, keepdims=True)
    if reload is None:
        xc = xT - m
        v = jnp.mean(xc * xc, axis=0, keepdims=True)
    else:
        xc = reload() - m
        v = jnp.mean(xc * xc, axis=0, keepdims=True)
        fence(v)
        xc = reload() - m
    hT = (xc * lax.rsqrt(v + EPS)) * _lanes(scale1p, TM) + _lanes(shift, TM)
    hT = jnp.concatenate([hT.astype(BF16), jnp.zeros((DP - D, TM), BF16)], axis=0)
    return hT.T


def _kernel(c_hbm, xT_hbm, wqkv_hbm, wo_hbm, w1_hbm, w2T_hbm, wmod_hbm, outT_hbm,
            c_v, xT_v, wqkv_v, wo_v, w1p, w2T_v, wmod_v, wT_f, wp, woT, modT, qkv, qkv0,
            hb1, hb2, x1T, ost, zsem, sems):
    def cp(src, dst, k):
        return pltpu.make_async_copy(src, dst, sems.at[k])

    def cp_x(b0, b1, k):
        return cp(xT_hbm.at[:, b0 * TM:b1 * TM], xT_v.at[:, b0 * TM:b1 * TM], k)

    g_wq = [cp(wqkv_hbm.at[:, 0:640], wqkv_v.at[:, 0:640], 0)]
    g_mod0 = [cp(c_hbm, c_v, 1), cp(wmod_hbm.at[:, 0:1152], wmod_v.at[:, 0:1152], 2)]
    g_x0 = [cp_x(0, 1, 3)]
    g_x1 = [cp_x(1, 4, 4)]
    g_wkv = [cp(wqkv_hbm.at[:, 640:1728], wqkv_v.at[:, 640:1728], 5), cp_x(4, 5, 6)]
    g_mid = [cp_x(5, NB, 7), cp(wo_hbm, wo_v, 8), cp(wmod_hbm.at[:, 1152:3456], wmod_v.at[:, 1152:3456], 9)]
    g_ffn = [cp(w1_hbm, w1p.at[0:D, :], 10), cp(w2T_hbm, w2T_v, 11)]
    for g in (g_wq, g_mod0, g_x0, g_x1, g_wkv, g_mid, g_ffn):
        for dma in g:
            dma.start()

    def wait(g):
        for dma in g:
            dma.wait()

    w1p[D:DP, :] = jnp.zeros((DP - D, DFF), BF16)
    for j in KVT:
        for p in range(4):
            rows = HALO + (8 if p else 0)
            qkv0[_kv_slab(j, p), 0:rows, :] = jnp.zeros((rows, 128), F32)
    wp[:, 128 * 12 + 64:128 * 13, :] = jnp.zeros((5, 64, 128), BF16)

    def w_transpose(c0, c1):
        for j in range(5):
            lo = 128 * j
            n = min(128, D - lo)
            blk = wqkv_v[lo:lo + n, c0:c1]
            if n < 128:
                blk = jnp.concatenate([blk, jnp.zeros((128 - n, c1 - c0), BF16)], axis=0)
            wT_f[j, c0:c1, :] = blk.T.astype(F32)

    def w_regroup(part):
        for d in range(DH):
            r = _qkv_row(part, d)
            for j in range(5):
                wp[j, r:r + 32, :] = wT_f.at[j][pl.ds(D * part + d, 32, stride=DH), :].astype(BF16)

    def prep_wo():
        for t in range(5):
            lo = 128 * t
            n = min(128, D - lo)
            wT_f[t, 0:D, 0:n] = wo_v[:, lo:lo + n].astype(F32)
            parts = [wT_f.at[t][pl.ds(d, 32, stride=DH), 0:n] for d in range(16)]
            parts.append(jnp.zeros((64, n), F32))
            parts += [wT_f.at[t][pl.ds(d, 32, stride=DH), 0:n] for d in (16, 17)]
            woT[lo:lo + n, :] = jnp.concatenate(parts, axis=0).astype(BF16).T

    def mod_tiles(s16, t0, t1):
        m = jnp.dot(s16, wmod_v[:, 128 * t0:128 * t1], preferred_element_type=F32)
        for t in range(t1 - t0):
            n0 = 128 * (t0 + t)
            col = jnp.broadcast_to(m[0:1, 128 * t:128 * t + 128], (128, 128)).T
            if (n0 < 2 * D and n0 + 128 > D) or (n0 < 5 * D and n0 + 128 > 4 * D):
                rid = n0 + lax.broadcasted_iota(jnp.int32, (128, 128), 0)
                is_scale = ((rid >= D) & (rid < 2 * D)) | ((rid >= 4 * D) & (rid < 5 * D))
                col = jnp.where(is_scale, col + 1.0, col)
            modT[n0:n0 + 128, :] = col

    def mod(k):
        return modT[k * D:(k + 1) * D, :]

    def ln_a(i):
        hb1[i] = _ln_mod(xT_v[:, i * TM:(i + 1) * TM].astype(F32), mod(1), mod(0))

    def mm_a(i, tiles, between=None):
        h = hb1[i]
        for j in tiles:
            wt = jnp.concatenate([wp[k, 128 * j:128 * j + 128, :] for k in range(5)], axis=1)
            r = _nt_dot(h, wt)
            if j in QT:
                r = r * (DH ** -0.5 * LOG2E)
            for p in range(4 if j in KVT else 1):
                if i == 0:
                    qkv0[_kv_slab(j, p), HALO + 2 * p:HALO + TM + 2 * p, :] = r
                    if j in KVT:
                        qkv[_kv_slab(j, p), TM + 2 * p:HALO + TM + 2 * p, :] = r[TM - HALO:TM, :]
                else:
                    qkv[_kv_slab(j, p), HALO + i * TM + 2 * p:HALO + (i + 1) * TM + 2 * p, :] = r
            if between is not None:
                between()

    def stage_b(i, buf, obase):
        for ch in range(TM // NA):
            t0 = i * TM + ch * NA
            r0 = HALO + t0
            if not isinstance(i, int):
                r0 = pl.multiple_of(r0, 8)

            def win(j, w):
                return buf[_kv_slab(j, w % 4), pl.ds(r0 - 8 * (w // 4), NA), :]

            qs = [buf[j, pl.ds(r0, NA), :] for j in QT]
            logits = []
            for w in range(W):
                acc = None
                for qi, j in enumerate(KT):
                    prod = qs[qi] * win(j, w)
                    acc = prod if acc is None else acc + prod
                acc = acc + pltpu.roll(acc, 64, 1)
                acc = acc + pltpu.roll(acc, 32, 1)
                if ch * NA < DIL * w:
                    tok = t0 + lax.broadcasted_iota(jnp.int32, (NA, 128), 0)
                    acc = jnp.where(tok >= DIL * w, acc, -1e9 * LOG2E)
                logits.append(acc)
            m = logits[0]
            for w in range(1, W):
                m = jnp.maximum(m, logits[w])
            ps = [jnp.exp2(l - m) for l in logits]
            den = ps[0]
            for w in range(1, W):
                den = den + ps[w]
            r = pltpu.reciprocal(den, approx=True)
            inv = r * (2.0 - den * r)
            for vi, j in enumerate(VT):
                acc = None
                for w in range(W):
                    prod = ps[w] * win(j, w)
                    acc = prod if acc is None else acc + prod
                buf[NQ + vi, pl.ds(obase + ch * NA, NA), :] = acc * inv

    def stage_c(i, slot, buf, obase):
        o = jnp.concatenate([buf[NQ + vi, pl.ds(obase, TM), :] for vi in range(5)], axis=1).astype(BF16)
        attnT = _nt_dot(woT[...], o)
        if isinstance(i, int):
            xT = xT_v[:, i * TM:(i + 1) * TM]
        else:
            xT = xT_v[:, pl.ds(pl.multiple_of(i * TM, 128), TM)]
        x1 = xT.astype(F32) + _lanes(mod(2), TM) * attnT
        x1T[slot, 0:D, :] = x1

        def fence(v):
            x1T[slot, D:D + 8, :] = jnp.broadcast_to(v, (8, TM))

        hb2[slot] = _ln_mod(x1, mod(4), mod(3), lambda: x1T[slot, 0:D, :], fence)

    def mm1(h, j):
        h1 = jnp.dot(h, w1p[:, j * FC:(j + 1) * FC], preferred_element_type=F32)
        return jnp.maximum(h1, 0.0).astype(BF16)

    nj = DFF // FC

    def stage_d(i, slot, hook_at, hook):
        h = hb2[slot]
        acc = None
        a_next = mm1(h, 0)
        for j in range(nj):
            a = a_next
            if j + 1 < nj:
                a_next = mm1(h, j + 1)
            if j == hook_at:
                hook()
            p = _nt_dot(w2T_v[:, j * FC:(j + 1) * FC], a)
            acc = p if acc is None else acc + p
        ost[i] = (x1T[slot, 0:D, :] + _lanes(mod(5), TM) * acc).astype(BF16)

    def cp_out(i):
        if isinstance(i, int):
            dst = outT_hbm.at[:, i * TM:(i + 1) * TM]
        else:
            dst = outT_hbm.at[:, pl.ds(pl.multiple_of(i * TM, 128), TM)]
        return cp(ost.at[i], dst, 12)

    wait(g_wq)
    w_transpose(0, 640)
    w_regroup(0)
    wait(g_mod0)
    cc = c_v[...].astype(F32)
    s16 = jnp.broadcast_to(cc * jax.nn.sigmoid(cc), (16, D)).astype(BF16)
    mod_tiles(s16, 0, 9)
    wait(g_x0)
    ln_a(0)
    mm_a(0, QT[:3])
    wait(g_x1)
    ln_a(1)
    ln_a(2)
    mm_a(0, QT[3:])
    mm_a(1, QT)
    ln_a(3)
    mm_a(2, QT)
    wait(g_wkv)
    w_transpose(640, 1728)
    w_regroup(1)
    w_regroup(2)
    mm_a(3, QT)
    ln_a(4)
    mm_a(0, KVT)
    mm_a(1, KVT)
    wait(g_mid)
    ob0 = pl.multiple_of(pl.semaphore_read(zsem) * 8, 8)
    stage_b(0, qkv0, ob0)
    prep_wo()
    todo = list(range(9, 27, 2))

    def mod_next():
        if todo:
            t = todo.pop(0)
            mod_tiles(s16, t, t + 2)

    mm_a(2, KVT, mod_next)
    mm_a(3, KVT, mod_next)
    for i in range(4, NB):
        if i > 4:
            ln_a(i)
        mm_a(i, tuple(range(NQ)))
        if i == 5:
            stage_c(0, 0, qkv0, ob0)
    wait(g_ffn)

    def body(i, carry):
        slot = i % 2
        ob = pl.multiple_of((1 - slot) * TM, 8)
        stage_b(i + 1, qkv, ob)
        stage_d(i, slot, 7, lambda: stage_c(i + 1, 1 - slot, qkv, ob))
        cp_out(i).start()
        return carry

    lax.fori_loop(0, NB - 1, body, 0)

    last = NB - 1
    slot = last % 2
    h = hb2[slot]

    def cp_half(u):
        lo = last * TM + 128 * u
        return cp(ost.at[last, :, 128 * u:128 * u + 128], outT_hbm.at[:, lo:lo + 128], 13)

    accs = [None, None]
    a_next = mm1(h, 0)
    for j in range(nj):
        a = a_next
        if j + 1 < nj:
            a_next = mm1(h, j + 1)
        w2 = w2T_v[:, j * FC:(j + 1) * FC]
        if j + 1 < nj:
            p = _nt_dot(w2, a)
            for u in range(2):
                pu = p[:, 128 * u:128 * u + 128]
                accs[u] = pu if accs[u] is None else accs[u] + pu
        else:
            for u in range(2):
                accs[u] = accs[u] + _nt_dot(w2, a[128 * u:128 * u + 128, :])
                res = x1T[slot, 0:D, 128 * u:128 * u + 128] + mod(5) * accs[u]
                ost[last, :, 128 * u:128 * u + 128] = res.astype(BF16)
                cp_half(u).start()
    for i in range(NB - 1):
        cp_out(i).wait()
    for u in range(2):
        cp_half(u).wait()


@jax.jit
def pallas_adaLN_cond__sliding_local_dilated__dense_activation_relu__prompt_kernel(
    A_x: jax.Array,
    A_wqkv: jax.Array,
    A_wo: jax.Array,
    B_x: jax.Array,
    B_w1: jax.Array,
    B_w2: jax.Array,
    c: jax.Array,
    w_mod: jax.Array,
):
    del B_x
    any_spec = pl.BlockSpec(memory_space=pl.ANY)
    outT = pl.pallas_call(
        _kernel,
        in_specs=[any_spec] * 7,
        out_specs=any_spec,
        out_shape=jax.ShapeDtypeStruct((D, S), BF16),
        scratch_shapes=[
            pltpu.VMEM((1, D), BF16),
            pltpu.VMEM((D, S), BF16),
            pltpu.VMEM((D, 3 * D), BF16),
            pltpu.VMEM((D, D), BF16),
            pltpu.VMEM((DP, DFF), BF16),
            pltpu.VMEM((D, DFF), BF16),
            pltpu.VMEM((D, 6 * D), BF16),
            pltpu.VMEM((5, 3 * D, 128), F32),
            pltpu.VMEM((5, 128 * NQ, 128), BF16),
            pltpu.VMEM((D, DP), BF16),
            pltpu.VMEM((6 * D, 128), F32),
            pltpu.VMEM((NSL, HALO + S + 8, 128), F32),
            pltpu.VMEM((NSL, HALO + TM + 8, 128), F32),
            pltpu.VMEM((NB, TM, DP), BF16),
            pltpu.VMEM((2, TM, DP), BF16),
            pltpu.VMEM((2, D + 8, TM), F32),
            pltpu.VMEM((NB, D, TM), BF16),
            pltpu.SemaphoreType.REGULAR,
            pltpu.SemaphoreType.DMA((14,)),
        ],
        compiler_params=pltpu.CompilerParams(
            vmem_limit_bytes=100 * 1024 * 1024,
            flags={"XLA_TPU_EVENLY_DISTRIBUTE_CRITICAL_NODES": True},
            disable_bounds_checks=True,
            disable_semaphore_checks=True,
        ),
    )(c, A_x.reshape(S, D).T, A_wqkv, A_wo, B_w1, B_w2.T, w_mod)
    return outT.T.reshape(1, S, D)
```

```python
import math

import jax
import jax.numpy as jnp
import numpy as np
from jax import lax
from jax.experimental import pallas as pl
from jax.experimental.pallas import tpu as pltpu

S, D, DFF = 2048, 576, 4608
H, DH, W, DIL = 32, 18, 8, 2
EPS = 1e-5
DP = 640
TM = 256
NB = S // TM
FC = 512
NA = 16
HALO = 16
LOG2E = math.log2(math.e)
F32, BF16 = jnp.float32, jnp.bfloat16

NQ = 14
QT = (0, 1, 2, 3, 12)
KT = (4, 5, 6, 7, 13)
VT = (8, 9, 10, 11, 13)
KVT = (4, 5, 6, 7, 8, 9, 10, 11, 13)
NSL = NQ + 5 + 3 * len(KVT)


def _nt_dot(a, b):
    return lax.dot_general(a, b, (((1,), (1,)), ((), ())), preferred_element_type=F32)


def _qkv_row(part, d):
    if d < 16:
        return 128 * (4 * part + d // 4) + 32 * (d % 4)
    return (128 * 12, 128 * 13, 128 * 13 + 64)[part] + 32 * (d - 16)


def _kv_slab(j, p):
    return j if p == 0 else NQ + 5 + 3 * KVT.index(j) + (p - 1)


def _lanes(v, n):
    return jnp.concatenate([v] * (n // 128), axis=1)


def _ln_mod(xT, scale1p, shift, reload=None, fence=None):
    m = jnp.mean(xT, axis=0, keepdims=True)
    if reload is None:
        xc = xT - m
        v = jnp.mean(xc * xc, axis=0, keepdims=True)
    else:
        xc = reload() - m
        v = jnp.mean(xc * xc, axis=0, keepdims=True)
        fence(v)
        xc = reload() - m
    hT = (xc * lax.rsqrt(v + EPS)) * _lanes(scale1p, TM) + _lanes(shift, TM)
    hT = jnp.concatenate([hT.astype(BF16), jnp.zeros((DP - D, TM), BF16)], axis=0)
    return hT.T


def _kernel(off_hbm, c_hbm, xT_hbm, wqkv_hbm, wo_hbm, w1_hbm, w2T_hbm, wmod_hbm, outT_hbm,
            c_v, xT_v, wqkv_v, wo_v, w1p, w2T_v, wmod_v, wT_f, wp, woT, modT, qkv, qkv0,
            hb1, hb2, x1T, ost, off_s, sems):
    def cp(src, dst, k):
        return pltpu.make_async_copy(src, dst, sems.at[k])

    def cp_x(b0, b1, k):
        return cp(xT_hbm.at[:, b0 * TM:b1 * TM], xT_v.at[:, b0 * TM:b1 * TM], k)

    g_wq = [cp(wqkv_hbm.at[:, 0:640], wqkv_v.at[:, 0:640], 0)]
    g_mod0 = [cp(c_hbm, c_v, 1), cp(wmod_hbm.at[:, 0:1152], wmod_v.at[:, 0:1152], 2)]
    g_x0 = [cp_x(0, 1, 3)]
    g_x1 = [cp_x(1, 4, 4)]
    g_wkv = [cp(wqkv_hbm.at[:, 640:1728], wqkv_v.at[:, 640:1728], 5), cp_x(4, 5, 6)]
    g_mid = [cp_x(5, NB, 7), cp(wo_hbm, wo_v, 8), cp(off_hbm, off_s, 14), cp(wmod_hbm.at[:, 1152:3456], wmod_v.at[:, 1152:3456], 9)]
    g_ffn = [cp(w1_hbm, w1p.at[0:D, :], 10), cp(w2T_hbm, w2T_v, 11)]
    for g in (g_wq, g_mod0, g_x0, g_x1, g_wkv, g_mid, g_ffn):
        for dma in g:
            dma.start()

    def wait(g):
        for dma in g:
            dma.wait()

    w1p[D:DP, :] = jnp.zeros((DP - D, DFF), BF16)
    for j in KVT:
        for p in range(4):
            rows = HALO + (8 if p else 0)
            qkv0[_kv_slab(j, p), 0:rows, :] = jnp.zeros((rows, 128), F32)
    wp[:, 128 * 12 + 64:128 * 13, :] = jnp.zeros((5, 64, 128), BF16)

    def w_transpose(c0, c1):
        for j in range(5):
            lo = 128 * j
            n = min(128, D - lo)
            blk = wqkv_v[lo:lo + n, c0:c1]
            if n < 128:
                blk = jnp.concatenate([blk, jnp.zeros((128 - n, c1 - c0), BF16)], axis=0)
            wT_f[j, c0:c1, :] = blk.T.astype(F32)

    def w_regroup(part):
        for d in range(DH):
            r = _qkv_row(part, d)
            for j in range(5):
                wp[j, r:r + 32, :] = wT_f.at[j][pl.ds(D * part + d, 32, stride=DH), :].astype(BF16)

    def prep_wo():
        for t in range(5):
            lo = 128 * t
            n = min(128, D - lo)
            wT_f[t, 0:D, 0:n] = wo_v[:, lo:lo + n].astype(F32)
            parts = [wT_f.at[t][pl.ds(d, 32, stride=DH), 0:n] for d in range(16)]
            parts.append(jnp.zeros((64, n), F32))
            parts += [wT_f.at[t][pl.ds(d, 32, stride=DH), 0:n] for d in (16, 17)]
            woT[lo:lo + n, :] = jnp.concatenate(parts, axis=0).astype(BF16).T

    def mod_tiles(s16, t0, t1):
        m = jnp.dot(s16, wmod_v[:, 128 * t0:128 * t1], preferred_element_type=F32)
        for t in range(t1 - t0):
            n0 = 128 * (t0 + t)
            col = jnp.broadcast_to(m[0:1, 128 * t:128 * t + 128], (128, 128)).T
            if (n0 < 2 * D and n0 + 128 > D) or (n0 < 5 * D and n0 + 128 > 4 * D):
                rid = n0 + lax.broadcasted_iota(jnp.int32, (128, 128), 0)
                is_scale = ((rid >= D) & (rid < 2 * D)) | ((rid >= 4 * D) & (rid < 5 * D))
                col = jnp.where(is_scale, col + 1.0, col)
            modT[n0:n0 + 128, :] = col

    def mod(k):
        return modT[k * D:(k + 1) * D, :]

    def ln_a(i):
        hb1[i] = _ln_mod(xT_v[:, i * TM:(i + 1) * TM].astype(F32), mod(1), mod(0))

    def mm_a(i, tiles, between=None):
        h = hb1[i]
        for j in tiles:
            wt = jnp.concatenate([wp[k, 128 * j:128 * j + 128, :] for k in range(5)], axis=1)
            r = _nt_dot(h, wt)
            if j in QT:
                r = r * (DH ** -0.5 * LOG2E)
            for p in range(4 if j in KVT else 1):
                if i == 0:
                    qkv0[_kv_slab(j, p), HALO + 2 * p:HALO + TM + 2 * p, :] = r
                    if j in KVT:
                        qkv[_kv_slab(j, p), TM + 2 * p:HALO + TM + 2 * p, :] = r[TM - HALO:TM, :]
                else:
                    qkv[_kv_slab(j, p), HALO + i * TM + 2 * p:HALO + (i + 1) * TM + 2 * p, :] = r
            if between is not None:
                between()

    def stage_b(i, buf, obase):
        for ch in range(TM // NA):
            t0 = i * TM + ch * NA
            r0 = HALO + t0
            if not isinstance(i, int):
                r0 = pl.multiple_of(r0, 8)

            def win(j, w):
                return buf[_kv_slab(j, w % 4), pl.ds(r0 - 8 * (w // 4), NA), :]

            qs = [buf[j, pl.ds(r0, NA), :] for j in QT]
            logits = []
            for w in range(W):
                acc = None
                for qi, j in enumerate(KT):
                    prod = qs[qi] * win(j, w)
                    acc = prod if acc is None else acc + prod
                acc = acc + pltpu.roll(acc, 64, 1)
                acc = acc + pltpu.roll(acc, 32, 1)
                if ch * NA < DIL * w:
                    tok = t0 + lax.broadcasted_iota(jnp.int32, (NA, 128), 0)
                    acc = jnp.where(tok >= DIL * w, acc, -1e9 * LOG2E)
                logits.append(acc)
            m = logits[0]
            for w in range(1, W):
                m = jnp.maximum(m, logits[w])
            ps = [jnp.exp2(l - m) for l in logits]
            den = ps[0]
            for w in range(1, W):
                den = den + ps[w]
            r = pltpu.reciprocal(den, approx=True)
            inv = r * (2.0 - den * r)
            for vi, j in enumerate(VT):
                acc = None
                for w in range(W):
                    prod = ps[w] * win(j, w)
                    acc = prod if acc is None else acc + prod
                buf[NQ + vi, pl.ds(obase + ch * NA, NA), :] = acc * inv

    def stage_c(i, slot, buf, obase):
        o = jnp.concatenate([buf[NQ + vi, pl.ds(obase, TM), :] for vi in range(5)], axis=1).astype(BF16)
        attnT = _nt_dot(woT[...], o)
        if isinstance(i, int):
            xT = xT_v[:, i * TM:(i + 1) * TM]
        else:
            xT = xT_v[:, pl.ds(pl.multiple_of(i * TM, 128), TM)]
        x1 = xT.astype(F32) + _lanes(mod(2), TM) * attnT
        x1T[slot, 0:D, :] = x1

        def fence(v):
            x1T[slot, D:D + 8, :] = jnp.broadcast_to(v, (8, TM))

        hb2[slot] = _ln_mod(x1, mod(4), mod(3), lambda: x1T[slot, 0:D, :], fence)

    def mm1(h, j):
        h1 = jnp.dot(h, w1p[:, j * FC:(j + 1) * FC], preferred_element_type=F32)
        return jnp.maximum(h1, 0.0).astype(BF16)

    nj = DFF // FC

    def stage_d(i, slot, hook_at, hook):
        h = hb2[slot]
        acc = None
        a_next = mm1(h, 0)
        for j in range(nj):
            a = a_next
            if j + 1 < nj:
                a_next = mm1(h, j + 1)
            if j == hook_at:
                hook()
            p = _nt_dot(w2T_v[:, j * FC:(j + 1) * FC], a)
            acc = p if acc is None else acc + p
        ost[i] = (x1T[slot, 0:D, :] + _lanes(mod(5), TM) * acc).astype(BF16)

    def cp_out(i):
        if isinstance(i, int):
            dst = outT_hbm.at[:, i * TM:(i + 1) * TM]
        else:
            dst = outT_hbm.at[:, pl.ds(pl.multiple_of(i * TM, 128), TM)]
        return cp(ost.at[i], dst, 12)

    wait(g_wq)
    w_transpose(0, 640)
    w_regroup(0)
    wait(g_mod0)
    cc = c_v[...].astype(F32)
    s16 = jnp.broadcast_to(cc * jax.nn.sigmoid(cc), (16, D)).astype(BF16)
    mod_tiles(s16, 0, 9)
    wait(g_x0)
    ln_a(0)
    mm_a(0, QT[:3])
    wait(g_x1)
    ln_a(1)
    ln_a(2)
    mm_a(0, QT[3:])
    mm_a(1, QT)
    ln_a(3)
    mm_a(2, QT)
    wait(g_wkv)
    w_transpose(640, 1728)
    w_regroup(1)
    w_regroup(2)
    mm_a(3, QT)
    ln_a(4)
    mm_a(0, KVT)
    mm_a(1, KVT)
    wait(g_mid)
    ob0 = pl.multiple_of(off_s[0], 8)
    stage_b(0, qkv0, ob0)
    prep_wo()
    todo = list(range(9, 27, 2))

    def mod_next():
        if todo:
            t = todo.pop(0)
            mod_tiles(s16, t, t + 2)

    mm_a(2, KVT, mod_next)
    mm_a(3, KVT, mod_next)
    for i in range(4, NB):
        if i > 4:
            ln_a(i)
        mm_a(i, tuple(range(NQ)))
        if i == 5:
            stage_c(0, 0, qkv0, ob0)
    wait(g_ffn)

    def body(i, carry):
        slot = i % 2
        ob = pl.multiple_of((1 - slot) * TM, 8)
        stage_b(i + 1, qkv, ob)
        stage_d(i, slot, 7, lambda: stage_c(i + 1, 1 - slot, qkv, ob))
        cp_out(i).start()
        return carry

    lax.fori_loop(0, NB - 1, body, 0)

    last = NB - 1
    slot = last % 2
    h = hb2[slot]

    def cp_half(u):
        lo = last * TM + 128 * u
        return cp(ost.at[last, :, 128 * u:128 * u + 128], outT_hbm.at[:, lo:lo + 128], 13)

    accs = [None, None]
    a_next = mm1(h, 0)
    for j in range(nj):
        a = a_next
        if j + 1 < nj:
            a_next = mm1(h, j + 1)
        w2 = w2T_v[:, j * FC:(j + 1) * FC]
        if j + 1 < nj:
            p = _nt_dot(w2, a)
            for u in range(2):
                pu = p[:, 128 * u:128 * u + 128]
                accs[u] = pu if accs[u] is None else accs[u] + pu
        else:
            for u in range(2):
                accs[u] = accs[u] + _nt_dot(w2, a[128 * u:128 * u + 128, :])
                res = x1T[slot, 0:D, 128 * u:128 * u + 128] + mod(5) * accs[u]
                ost[last, :, 128 * u:128 * u + 128] = res.astype(BF16)
                cp_half(u).start()
    for i in range(NB - 1):
        cp_out(i).wait()
    for u in range(2):
        cp_half(u).wait()


@jax.jit
def pallas_adaLN_cond__sliding_local_dilated__dense_activation_relu__prompt_kernel(
    A_x: jax.Array,
    A_wqkv: jax.Array,
    A_wo: jax.Array,
    B_x: jax.Array,
    B_w1: jax.Array,
    B_w2: jax.Array,
    c: jax.Array,
    w_mod: jax.Array,
):
    del B_x
    any_spec = pl.BlockSpec(memory_space=pl.ANY)
    outT = pl.pallas_call(
        _kernel,
        in_specs=[any_spec] * 8,
        out_specs=any_spec,
        out_shape=jax.ShapeDtypeStruct((D, S), BF16),
        scratch_shapes=[
            pltpu.VMEM((1, D), BF16),
            pltpu.VMEM((D, S), BF16),
            pltpu.VMEM((D, 3 * D), BF16),
            pltpu.VMEM((D, D), BF16),
            pltpu.VMEM((DP, DFF), BF16),
            pltpu.VMEM((D, DFF), BF16),
            pltpu.VMEM((D, 6 * D), BF16),
            pltpu.VMEM((5, 3 * D, 128), F32),
            pltpu.VMEM((5, 128 * NQ, 128), BF16),
            pltpu.VMEM((D, DP), BF16),
            pltpu.VMEM((6 * D, 128), F32),
            pltpu.VMEM((NSL, HALO + S + 8, 128), F32),
            pltpu.VMEM((NSL, HALO + TM + 8, 128), F32),
            pltpu.VMEM((NB, TM, DP), BF16),
            pltpu.VMEM((2, TM, DP), BF16),
            pltpu.VMEM((2, D + 8, TM), F32),
            pltpu.VMEM((NB, D, TM), BF16),
            pltpu.SMEM((1,), jnp.int32),
            pltpu.SemaphoreType.DMA((15,)),
        ],
        compiler_params=pltpu.CompilerParams(
            vmem_limit_bytes=100 * 1024 * 1024,
            flags={"XLA_TPU_EVENLY_DISTRIBUTE_CRITICAL_NODES": True},
            disable_bounds_checks=True,
            disable_semaphore_checks=True,
        ),
    )(np.zeros((1,), np.int32), c, A_x.reshape(S, D).T, A_wqkv, A_wo, B_w1, B_w2.T, w_mod)
    return outT.T.reshape(1, S, D)
```

```python
import math

import jax
import jax.numpy as jnp
import numpy as np
from jax import lax
from jax.experimental import pallas as pl
from jax.experimental.pallas import tpu as pltpu

S, D, DFF = 2048, 576, 4608
H, DH, W, DIL = 32, 18, 8, 2
EPS = 1e-5
DP = 640
TM = 256
NB = S // TM
FC = 512
NA = 16
HALO = 16
LOG2E = math.log2(math.e)
F32, BF16 = jnp.float32, jnp.bfloat16

NQ = 14
QT = (0, 1, 2, 3, 12)
KT = (4, 5, 6, 7, 13)
VT = (8, 9, 10, 11, 13)
KVT = (4, 5, 6, 7, 8, 9, 10, 11, 13)
TAILS = -1
NSL = NQ + 5 + 3 * len(KVT)


def _nt_dot(a, b):
    return lax.dot_general(a, b, (((1,), (1,)), ((), ())), preferred_element_type=F32)


def _qkv_row(part, d):
    if d < 16:
        return 128 * (4 * part + d // 4) + 32 * (d % 4)
    return (128 * 12, 128 * 13, 128 * 13 + 64)[part] + 32 * (d - 16)


def _kv_slab(j, p):
    return j if p == 0 else NQ + 5 + 3 * KVT.index(j) + (p - 1)


def _lanes(v, n):
    return jnp.concatenate([v] * (n // 128), axis=1)


def _ln_mod(xT, scale1p, shift, reload=None, fence=None):
    m = jnp.mean(xT, axis=0, keepdims=True)
    if reload is None:
        xc = xT - m
        v = jnp.mean(xc * xc, axis=0, keepdims=True)
    else:
        xc = reload() - m
        v = jnp.mean(xc * xc, axis=0, keepdims=True)
        fence(v)
        xc = reload() - m
    hT = (xc * lax.rsqrt(v + EPS)) * _lanes(scale1p, TM) + _lanes(shift, TM)
    hT = jnp.concatenate([hT.astype(BF16), jnp.zeros((DP - D, TM), BF16)], axis=0)
    return hT.T


def _kernel(off_hbm, c_hbm, xT_hbm, wqkv_hbm, wo_hbm, w1_hbm, w2T_hbm, wmod_hbm, outT_hbm,
            c_v, xT_v, wqkv_v, wo_v, w1p, w2T_v, wmod_v, wT_f, wp, woT, modT, qkv, qkv0,
            hb1, hb2, x1T, ost, off_s, sems):
    def cp(src, dst, k):
        return pltpu.make_async_copy(src, dst, sems.at[k])

    def cp_x(b0, b1, k):
        return cp(xT_hbm.at[:, b0 * TM:b1 * TM], xT_v.at[:, b0 * TM:b1 * TM], k)

    g_wq = [cp(wqkv_hbm.at[:, 0:640], wqkv_v.at[:, 0:640], 0)]
    g_mod0 = [cp(c_hbm, c_v, 1), cp(wmod_hbm.at[:, 0:1152], wmod_v.at[:, 0:1152], 2)]
    g_x0 = [cp_x(0, 1, 3)]
    g_x1 = [cp_x(1, 4, 4)]
    g_wkv = [cp(wqkv_hbm.at[:, 640:1728], wqkv_v.at[:, 640:1728], 5), cp_x(4, 5, 6)]
    g_mid = [cp_x(5, NB, 7), cp(wo_hbm, wo_v, 8), cp(off_hbm, off_s, 14), cp(wmod_hbm.at[:, 1152:3456], wmod_v.at[:, 1152:3456], 9)]
    g_ffn = [cp(w1_hbm, w1p.at[0:D, :], 10), cp(w2T_hbm, w2T_v, 11)]
    for g in (g_wq, g_mod0, g_x0, g_x1, g_wkv, g_mid, g_ffn):
        for dma in g:
            dma.start()

    def wait(g):
        for dma in g:
            dma.wait()

    w1p[D:DP, :] = jnp.zeros((DP - D, DFF), BF16)
    for j in KVT:
        for p in range(4):
            rows = HALO + (8 if p else 0)
            qkv0[_kv_slab(j, p), 0:rows, :] = jnp.zeros((rows, 128), F32)
    wp[:, 128 * 12 + 64:128 * 13, :] = jnp.zeros((5, 64, 128), BF16)

    def w_transpose(c0, c1):
        for j in range(5):
            lo = 128 * j
            n = min(128, D - lo)
            blk = wqkv_v[lo:lo + n, c0:c1]
            if n < 128:
                blk = jnp.concatenate([blk, jnp.zeros((128 - n, c1 - c0), BF16)], axis=0)
            wT_f[j, c0:c1, :] = blk.T.astype(F32)

    def w_regroup(part):
        for d in range(DH):
            r = _qkv_row(part, d)
            for j in range(5):
                wp[j, r:r + 32, :] = wT_f.at[j][pl.ds(D * part + d, 32, stride=DH), :].astype(BF16)

    def prep_wo():
        for t in range(5):
            lo = 128 * t
            n = min(128, D - lo)
            wT_f[t, 0:D, 0:n] = wo_v[:, lo:lo + n].astype(F32)
            parts = [wT_f.at[t][pl.ds(d, 32, stride=DH), 0:n] for d in range(16)]
            parts.append(jnp.zeros((64, n), F32))
            parts += [wT_f.at[t][pl.ds(d, 32, stride=DH), 0:n] for d in (16, 17)]
            woT[lo:lo + n, :] = jnp.concatenate(parts, axis=0).astype(BF16).T

    def mod_tiles(s16, t0, t1):
        m = jnp.dot(s16, wmod_v[:, 128 * t0:128 * t1], preferred_element_type=F32)
        for t in range(t1 - t0):
            n0 = 128 * (t0 + t)
            col = jnp.broadcast_to(m[0:1, 128 * t:128 * t + 128], (128, 128)).T
            if (n0 < 2 * D and n0 + 128 > D) or (n0 < 5 * D and n0 + 128 > 4 * D):
                rid = n0 + lax.broadcasted_iota(jnp.int32, (128, 128), 0)
                is_scale = ((rid >= D) & (rid < 2 * D)) | ((rid >= 4 * D) & (rid < 5 * D))
                col = jnp.where(is_scale, col + 1.0, col)
            modT[n0:n0 + 128, :] = col

    def mod(k):
        return modT[k * D:(k + 1) * D, :]

    def ln_a(i):
        hb1[i] = _ln_mod(xT_v[:, i * TM:(i + 1) * TM].astype(F32), mod(1), mod(0))

    def put(i, j, r):
        for p in range(4 if j in KVT else 1):
            if i == 0:
                qkv0[_kv_slab(j, p), HALO + 2 * p:HALO + TM + 2 * p, :] = r
                if j in KVT:
                    qkv[_kv_slab(j, p), TM + 2 * p:HALO + TM + 2 * p, :] = r[TM - HALO:TM, :]
            else:
                qkv[_kv_slab(j, p), HALO + i * TM + 2 * p:HALO + (i + 1) * TM + 2 * p, :] = r

    qscale = DH ** -0.5 * LOG2E

    def mm_a(i, tiles, between=None):
        h = hb1[i]
        for j in tiles:
            if j == TAILS:
                wt = jnp.concatenate(
                    [jnp.concatenate([wp[k, 128 * 12:128 * 12 + 64, :], wp[k, 128 * 13:128 * 14, :]], axis=0)
                     for k in range(5)], axis=1)
                rT = _nt_dot(wt, h)
                put(i, 12, jnp.concatenate([rT[0:64] * qscale, jnp.zeros((64, TM), F32)], axis=0).T)
                put(i, 13, rT[64:192].T)
            else:
                wt = jnp.concatenate([wp[k, 128 * j:128 * j + 128, :] for k in range(5)], axis=1)
                r = _nt_dot(h, wt)
                put(i, j, r * qscale if j in QT else r)
            if between is not None:
                between()

    def stage_b(i, buf, obase):
        for ch in range(TM // NA):
            t0 = i * TM + ch * NA
            r0 = HALO + t0
            if not isinstance(i, int):
                r0 = pl.multiple_of(r0, 8)

            def win(j, w):
                return buf[_kv_slab(j, w % 4), pl.ds(r0 - 8 * (w // 4), NA), :]

            qs = [buf[j, pl.ds(r0, NA), :] for j in QT]
            logits = []
            for w in range(W):
                acc = None
                for qi, j in enumerate(KT):
                    prod = qs[qi] * win(j, w)
                    acc = prod if acc is None else acc + prod
                acc = acc + pltpu.roll(acc, 64, 1)
                acc = acc + pltpu.roll(acc, 32, 1)
                if ch * NA < DIL * w:
                    tok = t0 + lax.broadcasted_iota(jnp.int32, (NA, 128), 0)
                    acc = jnp.where(tok >= DIL * w, acc, -1e9 * LOG2E)
                logits.append(acc)
            m = logits[0]
            for w in range(1, W):
                m = jnp.maximum(m, logits[w])
            ps = [jnp.exp2(l - m) for l in logits]
            den = ps[0]
            for w in range(1, W):
                den = den + ps[w]
            r = pltpu.reciprocal(den, approx=True)
            inv = r * (2.0 - den * r)
            for vi, j in enumerate(VT):
                acc = None
                for w in range(W):
                    prod = ps[w] * win(j, w)
                    acc = prod if acc is None else acc + prod
                buf[NQ + vi, pl.ds(obase + ch * NA, NA), :] = acc * inv

    def stage_c(i, slot, buf, obase):
        o = jnp.concatenate([buf[NQ + vi, pl.ds(obase, TM), :] for vi in range(5)], axis=1).astype(BF16)
        attnT = _nt_dot(woT[...], o)
        if isinstance(i, int):
            xT = xT_v[:, i * TM:(i + 1) * TM]
        else:
            xT = xT_v[:, pl.ds(pl.multiple_of(i * TM, 128), TM)]
        x1 = xT.astype(F32) + _lanes(mod(2), TM) * attnT
        x1T[slot, 0:D, :] = x1

        def fence(v):
            x1T[slot, D:D + 8, :] = jnp.broadcast_to(v, (8, TM))

        hb2[slot] = _ln_mod(x1, mod(4), mod(3), lambda: x1T[slot, 0:D, :], fence)

    def mm1(h, j):
        h1 = jnp.dot(h, w1p[:, j * FC:(j + 1) * FC], preferred_element_type=F32)
        return jnp.maximum(h1, 0.0).astype(BF16)

    nj = DFF // FC

    def stage_d(i, slot, hook_at, hook):
        h = hb2[slot]
        acc = None
        a_next = mm1(h, 0)
        for j in range(nj):
            a = a_next
            if j + 1 < nj:
                a_next = mm1(h, j + 1)
            if j == hook_at:
                hook()
            p = _nt_dot(w2T_v[:, j * FC:(j + 1) * FC], a)
            acc = p if acc is None else acc + p
        ost[i] = (x1T[slot, 0:D, :] + _lanes(mod(5), TM) * acc).astype(BF16)

    def cp_out(i):
        if isinstance(i, int):
            dst = outT_hbm.at[:, i * TM:(i + 1) * TM]
        else:
            dst = outT_hbm.at[:, pl.ds(pl.multiple_of(i * TM, 128), TM)]
        return cp(ost.at[i], dst, 12)

    wait(g_wq)
    w_transpose(0, 640)
    w_regroup(0)
    wait(g_mod0)
    cc = c_v[...].astype(F32)
    s16 = jnp.broadcast_to(cc * jax.nn.sigmoid(cc), (16, D)).astype(BF16)
    mod_tiles(s16, 0, 9)
    wait(g_x0)
    ln_a(0)
    mm_a(0, QT[:3])
    wait(g_x1)
    ln_a(1)
    ln_a(2)
    mm_a(0, QT[3:])
    mm_a(1, QT[:4])
    ln_a(3)
    mm_a(2, QT[:4])
    wait(g_wkv)
    w_transpose(640, 1728)
    w_regroup(1)
    w_regroup(2)
    mm_a(3, QT[:4])
    ln_a(4)
    mm_a(0, KVT)
    mm_a(1, KVT[:8] + (TAILS,))
    wait(g_mid)
    ob0 = pl.multiple_of(off_s[0], 8)
    stage_b(0, qkv0, ob0)
    prep_wo()
    todo = list(range(9, 27, 2))

    def mod_next():
        if todo:
            t = todo.pop(0)
            mod_tiles(s16, t, t + 2)

    mm_a(2, KVT[:8] + (TAILS,), mod_next)
    mm_a(3, KVT[:8] + (TAILS,), mod_next)
    for i in range(4, NB):
        if i > 4:
            ln_a(i)
        mm_a(i, tuple(range(12)) + (TAILS,))
        if i == 5:
            stage_c(0, 0, qkv0, ob0)
    wait(g_ffn)

    def body(i, carry):
        slot = i % 2
        ob = pl.multiple_of((1 - slot) * TM, 8)
        stage_b(i + 1, qkv, ob)
        stage_d(i, slot, 7, lambda: stage_c(i + 1, 1 - slot, qkv, ob))
        cp_out(i).start()
        return carry

    lax.fori_loop(0, NB - 1, body, 0)

    last = NB - 1
    slot = last % 2
    h = hb2[slot]

    def cp_half(u):
        lo = last * TM + 128 * u
        return cp(ost.at[last, :, 128 * u:128 * u + 128], outT_hbm.at[:, lo:lo + 128], 13)

    accs = [None, None]
    a_next = mm1(h, 0)
    for j in range(nj):
        a = a_next
        if j + 1 < nj:
            a_next = mm1(h, j + 1)
        w2 = w2T_v[:, j * FC:(j + 1) * FC]
        if j + 1 < nj:
            p = _nt_dot(w2, a)
            for u in range(2):
                pu = p[:, 128 * u:128 * u + 128]
                accs[u] = pu if accs[u] is None else accs[u] + pu
        else:
            for u in range(2):
                accs[u] = accs[u] + _nt_dot(w2, a[128 * u:128 * u + 128, :])
                res = x1T[slot, 0:D, 128 * u:128 * u + 128] + mod(5) * accs[u]
                ost[last, :, 128 * u:128 * u + 128] = res.astype(BF16)
                cp_half(u).start()
    for i in range(NB - 1):
        cp_out(i).wait()
    for u in range(2):
        cp_half(u).wait()


@jax.jit
def pallas_adaLN_cond__sliding_local_dilated__dense_activation_relu__prompt_kernel(
    A_x: jax.Array,
    A_wqkv: jax.Array,
    A_wo: jax.Array,
    B_x: jax.Array,
    B_w1: jax.Array,
    B_w2: jax.Array,
    c: jax.Array,
    w_mod: jax.Array,
):
    del B_x
    any_spec = pl.BlockSpec(memory_space=pl.ANY)
    outT = pl.pallas_call(
        _kernel,
        in_specs=[any_spec] * 8,
        out_specs=any_spec,
        out_shape=jax.ShapeDtypeStruct((D, S), BF16),
        scratch_shapes=[
            pltpu.VMEM((1, D), BF16),
            pltpu.VMEM((D, S), BF16),
            pltpu.VMEM((D, 3 * D), BF16),
            pltpu.VMEM((D, D), BF16),
            pltpu.VMEM((DP, DFF), BF16),
            pltpu.VMEM((D, DFF), BF16),
            pltpu.VMEM((D, 6 * D), BF16),
            pltpu.VMEM((5, 3 * D, 128), F32),
            pltpu.VMEM((5, 128 * NQ, 128), BF16),
            pltpu.VMEM((D, DP), BF16),
            pltpu.VMEM((6 * D, 128), F32),
            pltpu.VMEM((NSL, HALO + S + 8, 128), F32),
            pltpu.VMEM((NSL, HALO + TM + 8, 128), F32),
            pltpu.VMEM((NB, TM, DP), BF16),
            pltpu.VMEM((2, TM, DP), BF16),
            pltpu.VMEM((2, D + 8, TM), F32),
            pltpu.VMEM((NB, D, TM), BF16),
            pltpu.SMEM((1,), jnp.int32),
            pltpu.SemaphoreType.DMA((15,)),
        ],
        compiler_params=pltpu.CompilerParams(
            vmem_limit_bytes=100 * 1024 * 1024,
            flags={"XLA_TPU_EVENLY_DISTRIBUTE_CRITICAL_NODES": True},
            disable_bounds_checks=True,
            disable_semaphore_checks=True,
        ),
    )(np.zeros((1,), np.int32), c, A_x.reshape(S, D).T, A_wqkv, A_wo, B_w1, B_w2.T, w_mod)
    return outT.T.reshape(1, S, D)
```

```python
import math

import jax
import jax.numpy as jnp
import numpy as np
from jax import lax
from jax.experimental import pallas as pl
from jax.experimental.pallas import tpu as pltpu

S, D, DFF = 2048, 576, 4608
H, DH, W, DIL = 32, 18, 8, 2
EPS = 1e-5
DP = 640
TM = 256
NB = S // TM
FC = 512
NA = 16
HALO = 16
LOG2E = math.log2(math.e)
F32, BF16 = jnp.float32, jnp.bfloat16

NQ = 14
QT = (0, 1, 2, 3, 12)
KT = (4, 5, 6, 7, 13)
VT = (8, 9, 10, 11, 13)
KVT = (4, 5, 6, 7, 8, 9, 10, 11, 13)
TAILS = -1
NSL = NQ + 5 + 3 * len(KVT)


def _nt_dot(a, b):
    return lax.dot_general(a, b, (((1,), (1,)), ((), ())), preferred_element_type=F32)


def _qkv_row(part, d):
    if d < 16:
        return 128 * (4 * part + d // 4) + 32 * (d % 4)
    return (128 * 12, 128 * 13, 128 * 13 + 64)[part] + 32 * (d - 16)


def _kv_slab(j, p):
    return j if p == 0 else NQ + 5 + 3 * KVT.index(j) + (p - 1)


def _lanes(v, n):
    return jnp.concatenate([v] * (n // 128), axis=1)


def _ln_mod(xT, scale1p, shift, reload=None, fence=None):
    m = jnp.mean(xT, axis=0, keepdims=True)
    if reload is None:
        xc = xT - m
        v = jnp.mean(xc * xc, axis=0, keepdims=True)
    else:
        xc = reload() - m
        v = jnp.mean(xc * xc, axis=0, keepdims=True)
        fence(v)
        xc = reload() - m
    hT = (xc * lax.rsqrt(v + EPS)) * _lanes(scale1p, TM) + _lanes(shift, TM)
    hT = jnp.concatenate([hT.astype(BF16), jnp.zeros((DP - D, TM), BF16)], axis=0)
    return hT.T


def _kernel(off_hbm, c_hbm, xT_hbm, wqkv_hbm, wo_hbm, w1_hbm, w2T_hbm, wmod_hbm, outT_hbm,
            c_v, xT_v, wqkv_v, wo_v, w1p, w2T_v, wmod_v, wT_f, wp, woT, modT, qkv, qkv0,
            hb1, hb2, x1T, ost, off_s, sems):
    def cp(src, dst, k):
        return pltpu.make_async_copy(src, dst, sems.at[k])

    def cp_x(b0, b1, k):
        return cp(xT_hbm.at[:, b0 * TM:b1 * TM], xT_v.at[:, b0 * TM:b1 * TM], k)

    g_wq = [cp(wqkv_hbm.at[:, 0:640], wqkv_v.at[:, 0:640], 0)]
    g_mod0 = [cp(c_hbm, c_v, 1), cp(wmod_hbm.at[:, 0:1152], wmod_v.at[:, 0:1152], 2)]
    g_x0 = [cp_x(0, 1, 3)]
    g_x1 = [cp_x(1, 4, 4)]
    g_wkv = [cp(wqkv_hbm.at[:, 640:1728], wqkv_v.at[:, 640:1728], 5), cp_x(4, 5, 6)]
    g_mid = [cp_x(5, NB, 7), cp(wo_hbm, wo_v, 8), cp(off_hbm, off_s, 14), cp(wmod_hbm.at[:, 1152:3456], wmod_v.at[:, 1152:3456], 9)]
    g_ffn = [cp(w1_hbm, w1p.at[0:D, :], 10), cp(w2T_hbm, w2T_v, 11)]
    for g in (g_wq, g_mod0, g_x0, g_x1, g_wkv, g_mid, g_ffn):
        for dma in g:
            dma.start()

    def wait(g):
        for dma in g:
            dma.wait()

    w1p[D:DP, :] = jnp.zeros((DP - D, DFF), BF16)
    for j in KVT:
        for p in range(4):
            rows = HALO + (8 if p else 0)
            qkv0[_kv_slab(j, p), 0:rows, :] = jnp.zeros((rows, 128), F32)
    wp[:, 128 * 12 + 64:128 * 13, :] = jnp.zeros((5, 64, 128), BF16)

    def w_transpose(c0, c1):
        for j in range(5):
            lo = 128 * j
            n = min(128, D - lo)
            blk = wqkv_v[lo:lo + n, c0:c1]
            if n < 128:
                blk = jnp.concatenate([blk, jnp.zeros((128 - n, c1 - c0), BF16)], axis=0)
            wT_f[j, c0:c1, :] = blk.T.astype(F32)

    def w_regroup(part):
        for d in range(DH):
            r = _qkv_row(part, d)
            for j in range(5):
                wp[j, r:r + 32, :] = wT_f.at[j][pl.ds(D * part + d, 32, stride=DH), :].astype(BF16)

    def prep_wo():
        for t in range(5):
            lo = 128 * t
            n = min(128, D - lo)
            wT_f[t, 0:D, 0:n] = wo_v[:, lo:lo + n].astype(F32)
            parts = [wT_f.at[t][pl.ds(d, 32, stride=DH), 0:n] for d in range(16)]
            parts.append(jnp.zeros((64, n), F32))
            parts += [wT_f.at[t][pl.ds(d, 32, stride=DH), 0:n] for d in (16, 17)]
            woT[lo:lo + n, :] = jnp.concatenate(parts, axis=0).astype(BF16).T

    def mod_tiles(s16, t0, t1):
        m = jnp.dot(s16, wmod_v[:, 128 * t0:128 * t1], preferred_element_type=F32)
        for t in range(t1 - t0):
            n0 = 128 * (t0 + t)
            col = jnp.broadcast_to(m[0:1, 128 * t:128 * t + 128], (128, 128)).T
            if (n0 < 2 * D and n0 + 128 > D) or (n0 < 5 * D and n0 + 128 > 4 * D):
                rid = n0 + lax.broadcasted_iota(jnp.int32, (128, 128), 0)
                is_scale = ((rid >= D) & (rid < 2 * D)) | ((rid >= 4 * D) & (rid < 5 * D))
                col = jnp.where(is_scale, col + 1.0, col)
            modT[n0:n0 + 128, :] = col

    def mod(k):
        return modT[k * D:(k + 1) * D, :]

    def ln_a(i):
        hb1[i] = _ln_mod(xT_v[:, i * TM:(i + 1) * TM].astype(F32), mod(1), mod(0))

    def put(i, j, r):
        for p in range(4 if j in KVT else 1):
            if i == 0:
                qkv0[_kv_slab(j, p), HALO + 2 * p:HALO + TM + 2 * p, :] = r
                if j in KVT:
                    qkv[_kv_slab(j, p), TM + 2 * p:HALO + TM + 2 * p, :] = r[TM - HALO:TM, :]
            else:
                qkv[_kv_slab(j, p), HALO + i * TM + 2 * p:HALO + (i + 1) * TM + 2 * p, :] = r

    qscale = DH ** -0.5 * LOG2E

    def mm_a(i, tiles, between=None):
        h = hb1[i]
        for j in tiles:
            if j == TAILS:
                wt = jnp.concatenate(
                    [jnp.concatenate([wp[k, 128 * 12:128 * 12 + 64, :], wp[k, 128 * 13:128 * 14, :]], axis=0)
                     for k in range(5)], axis=1)
                rT = _nt_dot(wt, h)
                put(i, 12, jnp.concatenate([rT[0:64] * qscale, jnp.zeros((64, TM), F32)], axis=0).T)
                put(i, 13, rT[64:192].T)
            else:
                wt = jnp.concatenate([wp[k, 128 * j:128 * j + 128, :] for k in range(5)], axis=1)
                r = _nt_dot(h, wt)
                put(i, j, r * qscale if j in QT else r)
            if between is not None:
                between()

    def stage_b(i, buf, obase):
        for ch in range(TM // NA):
            t0 = i * TM + ch * NA
            r0 = HALO + t0
            if not isinstance(i, int):
                r0 = pl.multiple_of(r0, 8)

            def win(j, w):
                return buf[_kv_slab(j, w % 4), pl.ds(r0 - 8 * (w // 4), NA), :]

            qs = [buf[j, pl.ds(r0, NA), :] for j in QT]
            logits = []
            for w in range(W):
                acc = None
                for qi, j in enumerate(KT):
                    prod = qs[qi] * win(j, w)
                    acc = prod if acc is None else acc + prod
                acc = acc + pltpu.roll(acc, 64, 1)
                acc = acc + pltpu.roll(acc, 32, 1)
                if ch * NA < DIL * w:
                    tok = t0 + lax.broadcasted_iota(jnp.int32, (NA, 128), 0)
                    acc = jnp.where(tok >= DIL * w, acc, -1e9 * LOG2E)
                logits.append(acc)
            m = logits[0]
            for w in range(1, W):
                m = jnp.maximum(m, logits[w])
            ps = [jnp.exp2(l - m) for l in logits]
            den = ps[0]
            for w in range(1, W):
                den = den + ps[w]
            r = pltpu.reciprocal(den, approx=True)
            inv = r * (2.0 - den * r)
            for vi, j in enumerate(VT):
                acc = None
                for w in range(W):
                    prod = ps[w] * win(j, w)
                    acc = prod if acc is None else acc + prod
                buf[NQ + vi, pl.ds(obase + ch * NA, NA), :] = acc * inv

    def stage_c(i, slot, buf, obase):
        o = jnp.concatenate([buf[NQ + vi, pl.ds(obase, TM), :] for vi in range(5)], axis=1).astype(BF16)
        attnT = _nt_dot(woT[...], o)
        if isinstance(i, int):
            xT = xT_v[:, i * TM:(i + 1) * TM]
        else:
            xT = xT_v[:, pl.ds(pl.multiple_of(i * TM, 128), TM)]
        x1 = xT.astype(F32) + _lanes(mod(2), TM) * attnT
        x1T[slot, 0:D, :] = x1

        def fence(v):
            x1T[slot, D:D + 8, :] = jnp.broadcast_to(v, (8, TM))

        hb2[slot] = _ln_mod(x1, mod(4), mod(3), lambda: x1T[slot, 0:D, :], fence)

    def mm1(h, j):
        h1 = jnp.dot(h, w1p[:, j * FC:(j + 1) * FC], preferred_element_type=F32)
        return jnp.maximum(h1, 0.0).astype(BF16)

    nj = DFF // FC

    def stage_d(i, slot, hook_at, hook):
        h = hb2[slot]
        acc = None
        a_next = mm1(h, 0)
        for j in range(nj):
            a = a_next
            if j + 1 < nj:
                a_next = mm1(h, j + 1)
            if j == hook_at:
                hook()
            p = _nt_dot(w2T_v[:, j * FC:(j + 1) * FC], a)
            acc = p if acc is None else acc + p
        ost[i] = (x1T[slot, 0:D, :] + _lanes(mod(5), TM) * acc).astype(BF16)

    def cp_out(i):
        if isinstance(i, int):
            dst = outT_hbm.at[:, i * TM:(i + 1) * TM]
        else:
            dst = outT_hbm.at[:, pl.ds(pl.multiple_of(i * TM, 128), TM)]
        return cp(ost.at[i], dst, 12)

    wait(g_wq)
    w_transpose(0, 640)
    w_regroup(0)
    wait(g_mod0)
    cc = c_v[...].astype(F32)
    s16 = jnp.broadcast_to(cc * jax.nn.sigmoid(cc), (16, D)).astype(BF16)
    mod_tiles(s16, 0, 9)
    wait(g_x0)
    ln_a(0)
    mm_a(0, QT[:3])
    wait(g_x1)
    ln_a(1)
    ln_a(2)
    mm_a(0, QT[3:])
    mm_a(1, QT[:4])
    ln_a(3)
    mm_a(2, QT[:4])
    wait(g_wkv)
    w_transpose(640, 1728)
    w_regroup(1)
    w_regroup(2)
    mm_a(3, QT[:4])
    ln_a(4)
    mm_a(0, KVT)
    mm_a(1, KVT[:4] + (TAILS,) + KVT[4:8])
    wait(g_mid)
    ob0 = pl.multiple_of(off_s[0], 8)
    stage_b(0, qkv0, ob0)
    prep_wo()
    todo = list(range(9, 27, 2))

    def mod_next():
        if todo:
            t = todo.pop(0)
            mod_tiles(s16, t, t + 2)

    mm_a(2, KVT[:4] + (TAILS,) + KVT[4:8], mod_next)
    mm_a(3, KVT[:4] + (TAILS,) + KVT[4:8], mod_next)
    for i in range(4, NB):
        if i > 4:
            ln_a(i)
        mm_a(i, tuple(range(4)) + (TAILS,) + tuple(range(4, 12)))
        if i == 5:
            stage_c(0, 0, qkv0, ob0)
    wait(g_ffn)

    def body(i, carry):
        slot = i % 2
        ob = pl.multiple_of((1 - slot) * TM, 8)
        stage_b(i + 1, qkv, ob)
        stage_d(i, slot, 7, lambda: stage_c(i + 1, 1 - slot, qkv, ob))
        cp_out(i).start()
        return carry

    lax.fori_loop(0, NB - 1, body, 0)

    last = NB - 1
    slot = last % 2
    h = hb2[slot]

    def cp_half(u):
        lo = last * TM + 128 * u
        return cp(ost.at[last, :, 128 * u:128 * u + 128], outT_hbm.at[:, lo:lo + 128], 13)

    accs = [None, None]
    a_next = mm1(h, 0)
    for j in range(nj):
        a = a_next
        if j + 1 < nj:
            a_next = mm1(h, j + 1)
        w2 = w2T_v[:, j * FC:(j + 1) * FC]
        if j + 1 < nj:
            p = _nt_dot(w2, a)
            for u in range(2):
                pu = p[:, 128 * u:128 * u + 128]
                accs[u] = pu if accs[u] is None else accs[u] + pu
        else:
            for u in range(2):
                accs[u] = accs[u] + _nt_dot(w2, a[128 * u:128 * u + 128, :])
                res = x1T[slot, 0:D, 128 * u:128 * u + 128] + mod(5) * accs[u]
                ost[last, :, 128 * u:128 * u + 128] = res.astype(BF16)
                cp_half(u).start()
    for i in range(NB - 1):
        cp_out(i).wait()
    for u in range(2):
        cp_half(u).wait()


@jax.jit
def pallas_adaLN_cond__sliding_local_dilated__dense_activation_relu__prompt_kernel(
    A_x: jax.Array,
    A_wqkv: jax.Array,
    A_wo: jax.Array,
    B_x: jax.Array,
    B_w1: jax.Array,
    B_w2: jax.Array,
    c: jax.Array,
    w_mod: jax.Array,
):
    del B_x
    any_spec = pl.BlockSpec(memory_space=pl.ANY)
    outT = pl.pallas_call(
        _kernel,
        in_specs=[any_spec] * 8,
        out_specs=any_spec,
        out_shape=jax.ShapeDtypeStruct((D, S), BF16),
        scratch_shapes=[
            pltpu.VMEM((1, D), BF16),
            pltpu.VMEM((D, S), BF16),
            pltpu.VMEM((D, 3 * D), BF16),
            pltpu.VMEM((D, D), BF16),
            pltpu.VMEM((DP, DFF), BF16),
            pltpu.VMEM((D, DFF), BF16),
            pltpu.VMEM((D, 6 * D), BF16),
            pltpu.VMEM((5, 3 * D, 128), F32),
            pltpu.VMEM((5, 128 * NQ, 128), BF16),
            pltpu.VMEM((D, DP), BF16),
            pltpu.VMEM((6 * D, 128), F32),
            pltpu.VMEM((NSL, HALO + S + 8, 128), F32),
            pltpu.VMEM((NSL, HALO + TM + 8, 128), F32),
            pltpu.VMEM((NB, TM, DP), BF16),
            pltpu.VMEM((2, TM, DP), BF16),
            pltpu.VMEM((2, D + 8, TM), F32),
            pltpu.VMEM((NB, D, TM), BF16),
            pltpu.SMEM((1,), jnp.int32),
            pltpu.SemaphoreType.DMA((15,)),
        ],
        compiler_params=pltpu.CompilerParams(
            vmem_limit_bytes=100 * 1024 * 1024,
            flags={"XLA_TPU_EVENLY_DISTRIBUTE_CRITICAL_NODES": True},
            disable_bounds_checks=True,
            disable_semaphore_checks=True,
        ),
    )(np.zeros((1,), np.int32), c, A_x.reshape(S, D).T, A_wqkv, A_wo, B_w1, B_w2.T, w_mod)
    return outT.T.reshape(1, S, D)
```
